```python
import os as _os
_os.environ.setdefault("JAX_PLATFORMS", "cpu")
import jax
import jax.numpy as jnp

def _softmax(x, axis=-1):
    return jax.nn.softmax(x, axis=axis)
def _gelu(x):
    return jax.nn.gelu(x, approximate=True)
def _silu(x):
    return jax.nn.silu(x)
def _sigmoid(x):
    return jax.nn.sigmoid(x)
def _layernorm(x, axis=-1, eps=1e-5):
    m = jnp.mean(x, axis=axis, keepdims=True)
    v = jnp.var(x, axis=axis, keepdims=True)
    return (x - m) / jnp.sqrt(v + eps)
def _scatter_add(tgt, idx, src, axis=0):
    return tgt.at[idx].add(src)
def _segment_sum(src, seg, n):
    return jax.ops.segment_sum(src, seg, n)
class _Rng:
    def __init__(self, key):
        self._k = key
    def _next(self):
        self._k, sub = jax.random.split(self._k)
        return sub
    def normal(self, shape):
        return jax.random.normal(self._next(), shape, dtype=jnp.bfloat16)
    def randint(self, lo, hi, shape):
        return jax.random.randint(self._next(), shape, lo, hi, dtype=jnp.int32)
    def uniform(self, shape, lo=0.0, hi=1.0):
        return jax.random.uniform(self._next(), shape, jnp.bfloat16, lo, hi)
    def permutation(self, n):
        return jax.random.permutation(self._next(), n)


kernel_name = 'interleave_layers__grouped_kv_mqa__sliding_block__prompt'

def setup_inputs():
    _rng = _Rng(jax.random.key(int.from_bytes(__import__("os").urandom(4), "little")))
    _w = (lambda a: (lambda t: t.astype(jnp.bfloat16) if jnp.issubdtype(t.dtype, jnp.floating) else t)(jnp.asarray(a)))
    def _A_setup():
        B, S, D, H = 1, 2048, 448, 16
        Dh = D // H
        return {
            "x": _w((lambda *s: _rng.normal(s) * 0.05)(B, S, D)),
            "wq": _w((lambda *s: _rng.normal(s) * 0.05)(D, H * Dh)),
            "wk": _w((lambda *s: _rng.normal(s) * 0.05)(D, Dh)),
            "wv": _w((lambda *s: _rng.normal(s) * 0.05)(D, Dh)),
            "wo": _w((lambda *s: _rng.normal(s) * 0.05)(H * Dh, D)),
        }
    _A_in = _A_setup()

    def _B_setup():
        B, S, D = 1, 2048, 448
        return {
            "x": _w((lambda *s: _rng.normal(s) * 0.05)(B, S, D)),
            "wqkv": _w((lambda *s: _rng.normal(s) * 0.05)(D, 3 * D)),
            "wo": _w((lambda *s: _rng.normal(s) * 0.05)(D, D)),
        }
    _B_in = _B_setup()

    return {
        "A_x": _A_in["x"],
        "A_wq": _A_in["wq"],
        "A_wk": _A_in["wk"],
        "A_wv": _A_in["wv"],
        "A_wo": _A_in["wo"],
        "B_x": _B_in["x"],
        "B_wqkv": _B_in["wqkv"],
        "B_wo": _B_in["wo"],
    }

def reference(A_x, A_wq, A_wk, A_wv, A_wo, B_x, B_wqkv, B_wo):
    def _A_ref(x, wq, wk, wv, wo):
        B, S, D = x.shape
        H = 16
        Dh = D // H
        q = (lambda x, *d: x.transpose(*d))((x @ wq).reshape(B, S, H, Dh), 0, 2, 1, 3)
        k = x @ wk
        v = x @ wv
        scores = jnp.einsum("bhqd,bkd->bhqk", q, k) * (Dh ** -0.5)
        p = _softmax(scores, axis=-1)
        o = jnp.einsum("bhqk,bkd->bhqd", p, v)
        return (lambda x, *d: x.transpose(*d))(o, 0, 2, 1, 3).reshape(B, S, H * Dh) @ wo

    def _B_ref(x, wqkv, wo):
        B, S, D = x.shape
        H = 16; Dh = D // H; W = 256
        qkv = (lambda x, *d: x.transpose(*d))((x @ wqkv).reshape(B, S, 3, H, Dh), 2, 0, 3, 1, 4)
        q, k, v = qkv[0], qkv[1], qkv[2]
        scores = jnp.einsum("bhqd,bhkd->bhqk", q, k) * (Dh ** -0.5)
        idx = jnp.arange(S)
        mask = (idx[:, None] - idx[None, :] >= 0) & (idx[:, None] - idx[None, :] < W)
        scores = jnp.where(mask[None, None], scores, -1e9)
        p = _softmax(scores, axis=-1)
        o = jnp.einsum("bhqk,bhkd->bhqd", p, v)
        return (lambda x, *d: x.transpose(*d))(o, 0, 2, 1, 3).reshape(B, S, D) @ wo

    x = A_x
    x = x + _A_ref(_layernorm(x, axis=-1), A_wq, A_wk, A_wv, A_wo)
    x = x + _B_ref(_layernorm(x, axis=-1), B_wqkv, B_wo)
    x = x + _A_ref(_layernorm(x, axis=-1), A_wq, A_wk, A_wv, A_wo)
    x = x + _B_ref(_layernorm(x, axis=-1), B_wqkv, B_wo)
    return x
```

```python
import functools

import jax
import jax.numpy as jnp
from jax import lax
import jax.experimental.pallas as pl
import jax.experimental.pallas.tpu as pltpu

S = 2048
D = 448
H = 16
DH = 28
DP = 32
HP = H * DP
W = 256
LB = 128
NB = S // LB
EPS = 1e-5
NEG = -1e30
QSCALE = (DH ** -0.5) * 1.4426950408889634

A_TQ = 256
A_CK = 512
A_NH = 4
A_NC = S // A_CK
A_NIT = (S // A_TQ) * H
P_TB = 512
P_NB = P_TB // LB

F32 = jnp.float32
BF16 = jnp.bfloat16


def _dot(a, b):
    return jnp.dot(a, b, preferred_element_type=F32)


def _kernel(xT_in, wa_in, wao_in, wb_in, wbo_in, out_ref,
            xT, qT, kA, vTA, kB, vTB, oT, sA, sB, bias, zero_s):
    zero_s[0] = 0

    for b in range(NB):
        xT[b] = xT_in[:, b * LB:(b + 1) * LB].astype(F32)

    r = lax.broadcasted_iota(jnp.int32, (3 * LB, LB), 0)
    c = lax.broadcasted_iota(jnp.int32, (3 * LB, LB), 1)
    for cls in range(3):
        d = c + cls * LB - r
        ok = jnp.logical_and(d >= 0, d < W)
        bias[cls] = jnp.where(ok, 0.0, NEG).astype(F32)

    ones_row = (lax.broadcasted_iota(jnp.int32, (DP, P_TB), 0) == DH)

    def layernorm_T(t):
        xs = jnp.concatenate([xT[t * P_NB + i] for i in range(P_NB)], axis=1)
        m = jnp.sum(xs, axis=0, keepdims=True) * (1.0 / D)
        xc = xs - m
        v = jnp.sum(xc * xc, axis=0, keepdims=True) * (1.0 / D)
        return (xc * lax.rsqrt(v + EPS)).astype(BF16)

    def out_proj(wo_ref):
        for t in range(S // P_TB):
            o = jnp.concatenate([oT[t * P_NB + i] for i in range(P_NB)], axis=1)
            y = _dot(wo_ref[...], o)
            for i in range(P_NB):
                xT[t * P_NB + i] = xT[t * P_NB + i] + y[:, i * LB:(i + 1) * LB]

    def proj_A():
        for t in range(S // P_TB):
            xn = layernorm_T(t)
            y = _dot(wa_in[...], xn)
            q = (y[:HP] * QSCALE).astype(BF16)
            for i in range(P_NB):
                qT[t * P_NB + i] = q[:, i * LB:(i + 1) * LB]
            kA[t * P_TB:(t + 1) * P_TB, :] = y[HP:HP + DP].T.astype(BF16)
            v = jnp.where(ones_row, 1.0, y[HP + DP:])
            vTA[:, t * P_TB:(t + 1) * P_TB] = v.astype(BF16)

    def attn_A():
        nq = A_TQ // LB

        def q_blk(it):
            qb = (it // H) * nq
            row = pl.multiple_of((it % H) * DP, DP)
            return jnp.concatenate([qT[qb + i, pl.ds(row, DP), :] for i in range(nq)], axis=1)

        def qk_chunk(q, s_ref, ci, m):
            s = _dot(kA[ci * A_CK:(ci + 1) * A_CK, :], q)
            s_ref[0, ci * A_CK:(ci + 1) * A_CK, 0:A_TQ] = s
            return jnp.maximum(m, jnp.max(s.reshape(A_CK // 8, 8, A_TQ), axis=0))

        def pv_chunk(s_ref, z, ci, mrow, acc):
            s = s_ref[z, ci * A_CK:(ci + 1) * A_CK, 0:A_TQ]
            p = jnp.exp2(s - mrow).astype(BF16)
            return acc + _dot(vTA[:, ci * A_CK:(ci + 1) * A_CK], p)

        def finish(it, acc):
            qb = (it // H) * nq
            row = pl.multiple_of((it % H) * DP, DP)
            o = (acc * (1.0 / acc[DH:DH + 1, :])).astype(BF16)
            for i in range(nq):
                oT[qb + i, pl.ds(row, DP), :] = o[:, i * LB:(i + 1) * LB]

        neg = jnp.full((8, A_TQ), -jnp.inf, F32)
        q0 = q_blk(0)
        m = neg
        for ci in range(A_NC):
            m = qk_chunk(q0, sA, ci, m)
        m0 = jnp.max(m, axis=0, keepdims=True)

        def half(it, z, mrow, s_cur, s_nxt):
            qn = q_blk(jnp.minimum(it + 1, A_NIT - 1))
            m = neg
            acc = jnp.zeros((DP, A_TQ), F32)
            for ci in range(A_NC + 1):
                if ci < A_NC:
                    m = qk_chunk(qn, s_nxt, ci, m)
                if ci >= 1:
                    acc = pv_chunk(s_cur, z, ci - 1, mrow, acc)
            finish(it, acc)
            return jnp.max(m, axis=0, keepdims=True)

        def body(j, mrow):
            z = zero_s[0]
            for u in range(A_NH):
                if u % 2 == 0:
                    mrow = half(A_NH * j + u, z, mrow, sA, sB)
                else:
                    mrow = half(A_NH * j + u, z, mrow, sB, sA)
            return mrow

        lax.fori_loop(0, A_NIT // A_NH, body, m0)

    ones_rows_B = (lax.broadcasted_iota(jnp.int32, (HP, P_TB), 0) % DP == DH)

    def proj_B():
        for t in range(S // P_TB):
            xn = layernorm_T(t)
            yq = _dot(wb_in[0:HP, :], xn)
            q = (yq * QSCALE).astype(BF16)
            for i in range(P_NB):
                qT[t * P_NB + i] = q[:, i * LB:(i + 1) * LB]
            yk = _dot(wb_in[HP:2 * HP, :], xn)
            for g in range(4):
                kB[g, t * P_TB:(t + 1) * P_TB, :] = yk[g * LB:(g + 1) * LB, :].T.astype(BF16)
            yv = _dot(wb_in[2 * HP:3 * HP, :], xn)
            v = jnp.where(ones_rows_B, 1.0, yv).astype(BF16)
            for i in range(P_NB):
                vTB[t * P_NB + i] = v[:, i * LB:(i + 1) * LB]

    def attn_B():
        NIT = NB * 4
        KW = 3 * LB
        zq = jnp.zeros((DP, LB), BF16)

        def qk(it, s_ref):
            b = it // 4
            g = it % 4
            kb0 = jnp.maximum(b - 2, 0)
            qg = qT[b, pl.ds(pl.multiple_of(g * LB, LB), LB), :]
            cols = []
            for j in range(4):
                parts = [qg[jj * DP:(jj + 1) * DP] if jj == j else zq for jj in range(4)]
                cols.append(jnp.concatenate(parts, axis=0))
            wq = jnp.concatenate(cols, axis=1)
            k = kB[g, pl.ds(pl.multiple_of(kb0 * LB, LB), KW), :]
            s = _dot(k, wq)
            bi = bias[jnp.minimum(b, 2)]
            s = s + jnp.concatenate([bi] * 4, axis=1)
            s_ref[0, 0:KW, :] = s
            m = jnp.max(s.reshape(KW // 8, 8, 4 * LB), axis=0)
            return jnp.max(m, axis=0, keepdims=True)

        def pv(it, z, s_ref, mrow):
            b = it // 4
            g = it % 4
            kb0 = jnp.maximum(b - 2, 0)
            p = jnp.exp2(s_ref[z, 0:KW, :] - mrow).astype(BF16)
            for j in range(4):
                row = pl.multiple_of(g * LB + j * DP, DP)
                v = jnp.concatenate([vTB[kb0 + i, pl.ds(row, DP), :] for i in range(3)], axis=1)
                acc = _dot(v, p[:, j * LB:(j + 1) * LB])
                o = (acc * (1.0 / acc[DH:DH + 1, :])).astype(BF16)
                oT[b, pl.ds(row, DP), :] = o

        m0 = qk(0, sA)
        B_NH = 4

        def body(jj, mrow):
            z = zero_s[0]
            for u in range(B_NH):
                it = B_NH * jj + u
                s_cur, s_nxt = (sA, sB) if u % 2 == 0 else (sB, sA)
                mn = qk(jnp.minimum(it + 1, NIT - 1), s_nxt)
                pv(it, z, s_cur, mrow)
                mrow = mn
            return mrow

        lax.fori_loop(0, NIT // B_NH, body, m0)

    def rep(_, carry):
        proj_A()
        attn_A()
        out_proj(wao_in)
        proj_B()
        attn_B()
        out_proj(wbo_in)
        return carry

    lax.fori_loop(0, 2, rep, 0)

    for b in range(NB):
        out_ref[:, b * LB:(b + 1) * LB] = xT[b].astype(out_ref.dtype)


def _pad_heads_rows(wT, n):
    return jnp.pad(wT.reshape(n, DH, D), ((0, 0), (0, DP - DH), (0, 0))).reshape(n * DP, D)


@jax.jit
def pallas_interleave_layers__grouped_kv_mqa__sliding_block__prompt_kernel(
    A_x: jax.Array,
    A_wq: jax.Array,
    A_wk: jax.Array,
    A_wv: jax.Array,
    A_wo: jax.Array,
    B_x: jax.Array,
    B_wqkv: jax.Array,
    B_wo: jax.Array,
):
    del B_x
    xT = A_x[0].T
    wa = _pad_heads_rows(jnp.concatenate([A_wq, A_wk, A_wv], axis=1).T, H + 2)
    wao = _pad_heads_rows(A_wo, H).T
    wb = _pad_heads_rows(B_wqkv.T, 3 * H)
    wbo = _pad_heads_rows(B_wo, H).T

    outT = pl.pallas_call(
        _kernel,
        out_shape=jax.ShapeDtypeStruct((D, S), A_x.dtype),
        scratch_shapes=[
            pltpu.VMEM((NB, D, LB), F32),
            pltpu.VMEM((NB, HP, LB), BF16),
            pltpu.VMEM((S, DP), BF16),
            pltpu.VMEM((DP, S), BF16),
            pltpu.VMEM((4, S, LB), BF16),
            pltpu.VMEM((NB, HP, LB), BF16),
            pltpu.VMEM((NB, HP, LB), BF16),
            pltpu.VMEM((1, S, 4 * LB), F32),
            pltpu.VMEM((1, S, 4 * LB), F32),
            pltpu.VMEM((3, 3 * LB, LB), F32),
            pltpu.SMEM((1,), jnp.int32),
        ],
        compiler_params=pltpu.CompilerParams(vmem_limit_bytes=100 * 2**20),
    )(xT, wa, wao, wb, wbo)
    return outT.T[None]
```

```python
import functools

import jax
import jax.numpy as jnp
from jax import lax
import jax.experimental.pallas as pl
import jax.experimental.pallas.tpu as pltpu

S = 2048
D = 448
H = 16
DH = 28
DP = 32
HP = H * DP
W = 256
LB = 128
NB = S // LB
EPS = 1e-5
NEG = -1e30
QSCALE = (DH ** -0.5) * 1.4426950408889634

A_TQ = 256
A_CK = 512
A_NC = S // A_CK
A_NQ = A_TQ // LB
A_NH = 8
A_NIT = (S // A_TQ) * H
P_TB = 512
P_NB = P_TB // LB
P_NT = S // P_TB

F32 = jnp.float32
BF16 = jnp.bfloat16


def _dot(a, b):
    return jnp.dot(a, b, preferred_element_type=F32)


def _repitch(y, n_heads, fill):
    parts = []
    for h in range(n_heads):
        parts += [y[h * DH:(h + 1) * DH], fill]
    return jnp.concatenate(parts, axis=0)


def _kernel(xT_hbm, wq_hbm, wkT_hbm, wvT_hbm, woA_hbm, wqkv_hbm, woB_hbm, out_hbm,
            x_raw, wq_raw, wkT_raw, wvT_raw, woA_raw, wqkv_raw, woB_raw, out_stage,
            waT, woAT, wbT, woBT,
            xT, qT, kA, vTA, kB, vTB, oT, sA, sB, bias, zero_s, sems, osems):
    zero_s[0] = 0

    def x_copy(t):
        return pltpu.make_async_copy(xT_hbm.at[:, pl.ds(t * P_TB, P_TB)], x_raw.at[t], sems.at[t])

    w_copies = [
        pltpu.make_async_copy(src, dst, sems.at[P_NT + i])
        for i, (src, dst) in enumerate([
            (wq_hbm, wq_raw), (wkT_hbm, wkT_raw), (wvT_hbm, wvT_raw),
            (woA_hbm, woA_raw), (wqkv_hbm, wqkv_raw), (woB_hbm, woB_raw)])
    ]
    for cp in w_copies[:3]:
        cp.start()
    for t in range(P_NT):
        x_copy(t).start()
    for cp in w_copies[3:]:
        cp.start()

    r = lax.broadcasted_iota(jnp.int32, (3 * LB, LB), 0)
    c = lax.broadcasted_iota(jnp.int32, (3 * LB, LB), 1)
    for cls in range(3):
        d = c + cls * LB - r
        ok = jnp.logical_and(d >= 0, d < W)
        bias[cls] = jnp.where(ok, 0.0, NEG).astype(F32)

    zero_fill = jnp.zeros((DP - DH, P_TB), F32)
    one_fill = (lax.broadcasted_iota(jnp.int32, (DP - DH, P_TB), 0) == 0).astype(F32)

    def load_x(t):
        return jnp.concatenate([xT[t * P_NB + i] for i in range(P_NB)], axis=1)

    def store_x(t, xs):
        for i in range(P_NB):
            xT[t * P_NB + i] = xs[:, i * LB:(i + 1) * LB]

    def layernorm_T(xs):
        m = jnp.sum(xs, axis=0, keepdims=True) * (1.0 / D)
        xc = xs - m
        v = jnp.sum(xc * xc, axis=0, keepdims=True) * (1.0 / D)
        return (xc * lax.rsqrt(v + EPS)).astype(BF16)

    def out_proj(wo_ref, t):
        o = jnp.concatenate([oT[t * P_NB + i] for i in range(P_NB)], axis=1)
        return load_x(t) + _dot(wo_ref[...], o)

    def proj_A(t, xs):
        xn = layernorm_T(xs)
        y = _dot(waT[...], xn)
        q = _repitch(y[:D] * QSCALE, H, zero_fill).astype(BF16)
        for i in range(P_NB):
            qT[t * P_NB + i] = q[:, i * LB:(i + 1) * LB]
        kA[t * P_TB:(t + 1) * P_TB, :] = y[D:D + DP].T.astype(BF16)
        v = _repitch(y[D + DP:D + DP + DH], 1, one_fill)
        vTA[:, t * P_TB:(t + 1) * P_TB] = v.astype(BF16)

    def attn_A():
        neg = jnp.full((8, A_TQ), -jnp.inf, F32)

        def qk_chunk(q, s_ref, ci, m):
            s = _dot(kA[ci * A_CK:(ci + 1) * A_CK, :], q)
            s_ref[0, ci * A_CK:(ci + 1) * A_CK, 0:A_TQ] = s
            return jnp.maximum(m, jnp.max(s.reshape(A_CK // 8, 8, A_TQ), axis=0))

        def pv_chunk(s_ref, z, ci, mrow, acc):
            s = s_ref[z, ci * A_CK:(ci + 1) * A_CK, 0:A_TQ]
            p = jnp.exp2(s - mrow).astype(BF16)
            return acc + _dot(vTA[:, ci * A_CK:(ci + 1) * A_CK], p)

        def q_blk(it):
            qb = (it // H) * A_NQ
            row = pl.multiple_of((it % H) * DP, DP)
            return jnp.concatenate([qT[qb + i, pl.ds(row, DP), :] for i in range(A_NQ)], axis=1)

        def finish(it, acc):
            qb = (it // H) * A_NQ
            row = pl.multiple_of((it % H) * DP, DP)
            o = (acc * (1.0 / acc[DH:DH + 1, :])).astype(BF16)
            for i in range(A_NQ):
                oT[qb + i, pl.ds(row, DP), :] = o[:, i * LB:(i + 1) * LB]

        q0 = q_blk(0)
        m = neg
        for ci in range(A_NC):
            m = qk_chunk(q0, sA, ci, m)
        m0 = jnp.max(m, axis=0, keepdims=True)

        def half(it, z, mrow, s_cur, s_nxt):
            qn = q_blk(jnp.minimum(it + 1, A_NIT - 1))
            m = neg
            acc = jnp.zeros((DP, A_TQ), F32)
            for ci in range(A_NC + 1):
                if ci < A_NC:
                    m = qk_chunk(qn, s_nxt, ci, m)
                if ci >= 1:
                    acc = pv_chunk(s_cur, z, ci - 1, mrow, acc)
            finish(it, acc)
            return jnp.max(m, axis=0, keepdims=True)

        def body(j, mrow):
            z = zero_s[0]
            for u in range(A_NH):
                if u % 2 == 0:
                    mrow = half(A_NH * j + u, z, mrow, sA, sB)
                else:
                    mrow = half(A_NH * j + u, z, mrow, sB, sA)
            return mrow

        lax.fori_loop(0, A_NIT // A_NH, body, m0)

    def proj_B(t, xs):
        xn = layernorm_T(xs)
        yq = _dot(wbT[0:D, :], xn)
        q = _repitch(yq * QSCALE, H, zero_fill).astype(BF16)
        for i in range(P_NB):
            qT[t * P_NB + i] = q[:, i * LB:(i + 1) * LB]
        yk = _repitch(_dot(wbT[D:2 * D, :], xn), H, zero_fill)
        for g in range(4):
            kB[g, t * P_TB:(t + 1) * P_TB, :] = yk[g * LB:(g + 1) * LB, :].T.astype(BF16)
        v = _repitch(_dot(wbT[2 * D:3 * D, :], xn), H, one_fill).astype(BF16)
        for i in range(P_NB):
            vTB[t * P_NB + i] = v[:, i * LB:(i + 1) * LB]

    def attn_B():
        NIT = NB * 4
        KW = 3 * LB
        zq = jnp.zeros((DP, LB), BF16)

        def qk(it, s_ref):
            b = it // 4
            g = it % 4
            kb0 = jnp.maximum(b - 2, 0)
            qg = qT[b, pl.ds(pl.multiple_of(g * LB, LB), LB), :]
            cols = []
            for j in range(4):
                parts = [qg[jj * DP:(jj + 1) * DP] if jj == j else zq for jj in range(4)]
                cols.append(jnp.concatenate(parts, axis=0))
            wq = jnp.concatenate(cols, axis=1)
            k = kB[g, pl.ds(pl.multiple_of(kb0 * LB, LB), KW), :]
            s = _dot(k, wq)
            bi = bias[jnp.minimum(b, 2)]
            s = s + jnp.concatenate([bi] * 4, axis=1)
            s_ref[0, 0:KW, :] = s
            m = jnp.max(s.reshape(KW // 8, 8, 4 * LB), axis=0)
            return jnp.max(m, axis=0, keepdims=True)

        def pv(it, z, s_ref, mrow):
            b = it // 4
            g = it % 4
            kb0 = jnp.maximum(b - 2, 0)
            p = jnp.exp2(s_ref[z, 0:KW, :] - mrow).astype(BF16)
            for j in range(4):
                row = pl.multiple_of(g * LB + j * DP, DP)
                v = jnp.concatenate([vTB[kb0 + i, pl.ds(row, DP), :] for i in range(3)], axis=1)
                acc = _dot(v, p[:, j * LB:(j + 1) * LB])
                o = (acc * (1.0 / acc[DH:DH + 1, :])).astype(BF16)
                oT[b, pl.ds(row, DP), :] = o

        m0 = qk(0, sA)
        B_NH = 4

        def body(jj, mrow):
            z = zero_s[0]
            for u in range(B_NH):
                it = B_NH * jj + u
                s_cur, s_nxt = (sA, sB) if u % 2 == 0 else (sB, sA)
                mn = qk(jnp.minimum(it + 1, NIT - 1), s_nxt)
                pv(it, z, s_cur, mrow)
                mrow = mn
            return mrow

        lax.fori_loop(0, NIT // B_NH, body, m0)

    zpad = jnp.zeros((DP - DH, D), F32)
    for cp in w_copies[:3]:
        cp.wait()
    waT[0:D, :] = wq_raw[...].T
    waT[D:D + 2 * DP, :] = jnp.concatenate(
        [wkT_raw[...].astype(F32), zpad, wvT_raw[...].astype(F32), zpad], axis=0).astype(BF16)
    for t in range(P_NT):
        x_copy(t).wait()
        store_x(t, x_raw[t].astype(F32))
    w_copies[3].wait()

    def out_copy(t):
        return pltpu.make_async_copy(out_stage.at[t], out_hbm.at[:, pl.ds(t * P_TB, P_TB)], osems.at[t])

    def rep(r_idx, carry):
        woAT[...] = _repitch(woA_raw[...].astype(F32), H, zpad).astype(BF16).T
        for t in range(P_NT):
            proj_A(t, load_x(t))

        attn_A()

        @pl.when(r_idx == 0)
        def _():
            w_copies[4].wait()
            w_copies[5].wait()

        wbT[...] = wqkv_raw[...].T
        woBT[...] = _repitch(woB_raw[...].astype(F32), H, zpad).astype(BF16).T
        for t in range(P_NT):
            store_x(t, out_proj(woAT, t))
        for t in range(P_NT):
            proj_B(t, load_x(t))

        attn_B()

        @pl.when(r_idx == 1)
        def _():
            for t in range(P_NT):
                out_copy(t).wait()

        for t in range(P_NT):
            xs = out_proj(woBT, t)
            store_x(t, xs)
            out_stage[t] = xs.astype(out_stage.dtype)
            out_copy(t).start()
        return carry

    lax.fori_loop(0, 2, rep, 0)
    for t in range(P_NT):
        out_copy(t).wait()


@jax.jit
def pallas_interleave_layers__grouped_kv_mqa__sliding_block__prompt_kernel(
    A_x: jax.Array,
    A_wq: jax.Array,
    A_wk: jax.Array,
    A_wv: jax.Array,
    A_wo: jax.Array,
    B_x: jax.Array,
    B_wqkv: jax.Array,
    B_wo: jax.Array,
):
    del B_x
    any_spec = pl.BlockSpec(memory_space=pl.ANY)
    outT = pl.pallas_call(
        _kernel,
        out_shape=jax.ShapeDtypeStruct((D, S), A_x.dtype),
        in_specs=[any_spec] * 7,
        out_specs=any_spec,
        scratch_shapes=[
            pltpu.VMEM((P_NT, D, P_TB), BF16),
            pltpu.VMEM((D, D), BF16),
            pltpu.VMEM((DH, D), BF16),
            pltpu.VMEM((DH, D), BF16),
            pltpu.VMEM((D, D), BF16),
            pltpu.VMEM((D, 3 * D), BF16),
            pltpu.VMEM((D, D), BF16),
            pltpu.VMEM((P_NT, D, P_TB), BF16),
            pltpu.VMEM((D + 2 * DP, D), BF16),
            pltpu.VMEM((D, HP), BF16),
            pltpu.VMEM((3 * D, D), BF16),
            pltpu.VMEM((D, HP), BF16),
            pltpu.VMEM((NB, D, LB), F32),
            pltpu.VMEM((NB, HP, LB), BF16),
            pltpu.VMEM((S, DP), BF16),
            pltpu.VMEM((DP, S), BF16),
            pltpu.VMEM((4, S, LB), BF16),
            pltpu.VMEM((NB, HP, LB), BF16),
            pltpu.VMEM((NB, HP, LB), BF16),
            pltpu.VMEM((1, S, 4 * LB), F32),
            pltpu.VMEM((1, S, 4 * LB), F32),
            pltpu.VMEM((3, 3 * LB, LB), F32),
            pltpu.SMEM((1,), jnp.int32),
            pltpu.SemaphoreType.DMA((P_NT + 6,)),
            pltpu.SemaphoreType.DMA((P_NT,)),
        ],
        compiler_params=pltpu.CompilerParams(vmem_limit_bytes=100 * 2**20),
    )(A_x[0].T, A_wq, A_wk.T, A_wv.T, A_wo, B_wqkv, B_wo)
    return outT.T[None]
```

```python
import functools

import jax
import jax.numpy as jnp
from jax import lax
import jax.experimental.pallas as pl
import jax.experimental.pallas.tpu as pltpu

S = 2048
D = 448
H = 16
DH = 28
DP = 32
HP = H * DP
W = 256
LB = 128
NB = S // LB
EPS = 1e-5
NEG = -1e30
QSCALE = (DH ** -0.5) * 1.4426950408889634

A_TQ = 256
A_CK = 256
A_NC = S // A_CK
A_NQ = A_TQ // LB
A_NH = 18
A_NIT = (S // A_TQ) * H
P_TB = 512
P_NB = P_TB // LB
P_NT = S // P_TB
A_PROJ_CHUNKS = ((0, 1), (1, 3), (4, 4), (8, 4), (12, 4))

B_U = 4
B_SB = LB // B_U
B_RB = LB + B_SB
B_R = LB + B_RB
B_LEAD = 3

LAST_POS = 1
LAST_POS_B = 0

F32 = jnp.float32
U32 = jnp.uint32
BF16 = jnp.bfloat16


def _dot(a, b):
    return jnp.dot(a, b, preferred_element_type=F32)


def _lane(shape):
    return lax.broadcasted_iota(jnp.int32, shape, 1)


def _sel(mask_fn, a, b):
    au = pltpu.bitcast(a, U32)
    bu = jnp.zeros_like(au) if b is None else pltpu.bitcast(b, U32)
    return pltpu.bitcast(jnp.where(mask_fn(_lane(au.shape)), au, bu), BF16)


def _repitch(y, n_heads, fill):
    parts = []
    for h in range(n_heads):
        parts += [y[h * DH:(h + 1) * DH], fill]
    return jnp.concatenate(parts, axis=0)


def _kernel(xT_hbm, wq_hbm, wkT_hbm, wvT_hbm, woA_hbm, wqkv_hbm, woB_hbm, out_hbm,
            x_raw, wq_raw, wkT_raw, wvT_raw, woA_raw, wqkv_raw, woB_raw, out_stage,
            waT, woAT, wbT, woBT,
            xT, xnB, qT, kA, vTA, kB, vTB, oT, sA, sB, sC, sD, bias, zero_s, sems, osems):
    zero_s[0] = 0

    def x_copy(t):
        return pltpu.make_async_copy(xT_hbm.at[:, pl.ds(t * P_TB, P_TB)], x_raw.at[t], sems.at[t])

    w_copies = [
        pltpu.make_async_copy(src, dst, sems.at[P_NT + i])
        for i, (src, dst) in enumerate([
            (wq_hbm, wq_raw), (wkT_hbm, wkT_raw), (wvT_hbm, wvT_raw),
            (woA_hbm, woA_raw), (wqkv_hbm, wqkv_raw), (woB_hbm, woB_raw)])
    ]
    for cp in w_copies[:3]:
        cp.start()
    for t in range(P_NT):
        x_copy(t).start()

    r = lax.broadcasted_iota(jnp.int32, (B_RB, LB), 0)
    c = lax.broadcasted_iota(jnp.int32, (B_RB, LB), 1)
    use_new = (c // B_SB) >= (r // B_SB)
    ok = jnp.logical_or(jnp.logical_and(use_new, r <= c),
                        jnp.logical_and(jnp.logical_not(use_new), r - B_SB > c))
    bias[...] = jnp.where(ok, 0.0, NEG).astype(F32)
    null_k = jnp.where(_lane((2 * LB, LB)) % DP == DH, NEG, 0.0).astype(BF16)
    for h in range(H):
        kB[h, 0:2 * LB, :] = null_k
    vTB[0:2] = jnp.zeros((2, HP, LB), BF16)

    def fills(n):
        return (jnp.zeros((DP - DH, n), F32),
                (lax.broadcasted_iota(jnp.int32, (DP - DH, n), 0) == 0).astype(F32))

    zero_fill, one_fill = fills(P_TB)

    def load_x(t):
        return jnp.concatenate([xT[t * P_NB + i] for i in range(P_NB)], axis=1)

    def store_x(t, xs):
        for i in range(P_NB):
            xT[t * P_NB + i] = xs[:, i * LB:(i + 1) * LB]

    def layernorm_T(xs):
        m = jnp.sum(xs, axis=0, keepdims=True) * (1.0 / D)
        xc = xs - m
        v = jnp.sum(xc * xc, axis=0, keepdims=True) * (1.0 / D)
        return (xc * lax.rsqrt(v + EPS)).astype(BF16)

    def out_proj(wo_ref, t):
        o = jnp.concatenate([oT[t * P_NB + i] for i in range(P_NB)], axis=1)
        return load_x(t) + _dot(wo_ref[...], o)

    def proj_A(b0, nb):
        n = nb * LB
        zf, of = fills(n)
        xn = layernorm_T(jnp.concatenate([xT[b0 + i] for i in range(nb)], axis=1))
        y = _dot(waT[...], xn)
        q = _repitch(y[:D] * QSCALE, H, zf).astype(BF16)
        for i in range(nb):
            qT[b0 + i] = q[:, i * LB:(i + 1) * LB]
        kA[b0 * LB:b0 * LB + n, :] = y[D:D + DP].T.astype(BF16)
        v = _repitch(y[D + DP:D + DP + DH], 1, of)
        vTA[:, b0 * LB:b0 * LB + n] = v.astype(BF16)

    neg_A = jnp.full((8, A_TQ), -jnp.inf, F32)

    def qk_chunk(q, s_ref, ci, m):
        s = _dot(kA[ci * A_CK:(ci + 1) * A_CK, :], q)
        s_ref[0, ci * A_CK:(ci + 1) * A_CK, :] = s
        return jnp.maximum(m, jnp.max(s.reshape(A_CK // 8, 8, A_TQ), axis=0))

    def pv_chunk(s_ref, z, ci, mrow, acc):
        s = s_ref[z, ci * A_CK:(ci + 1) * A_CK, :]
        p = jnp.exp2(s - mrow).astype(BF16)
        return acc + _dot(vTA[:, ci * A_CK:(ci + 1) * A_CK], p)

    def a_index(it):
        if isinstance(it, int):
            return (it // H) * A_NQ, (it % H) * DP
        qb = lax.shift_right_logical(it, 4) * A_NQ
        return qb, pl.multiple_of((it & (H - 1)) * DP, DP)

    def q_blk(it):
        qb, row = a_index(it)
        return jnp.concatenate([qT[qb + i, pl.ds(row, DP), :] for i in range(A_NQ)], axis=1)

    def step_A(it, z, mrow, s_cur, s_nxt, last=False):
        qn = None if last else q_blk(it + 1)
        m = neg_A
        acc = jnp.zeros((DP, A_TQ), F32)
        for ci in range(A_NC + 1):
            if ci < A_NC and not last:
                m = qk_chunk(qn, s_nxt, ci, m)
            if ci >= 1:
                acc = pv_chunk(s_cur, z, ci - 1, mrow, acc)
        qb, row = a_index(it)
        o = (acc * (1.0 / acc[DH:DH + 1, :])).astype(BF16)
        for i in range(A_NQ):
            oT[qb + i, pl.ds(row, DP), :] = o[:, i * LB:(i + 1) * LB]
        return jnp.max(m, axis=0, keepdims=True)

    def attn_A_main():
        q0 = q_blk(0)
        m = neg_A
        for ci in range(A_NC):
            m = qk_chunk(q0, sA, ci, m)
        m0 = jnp.max(m, axis=0, keepdims=True)
        m1 = step_A(0, zero_s[0], m0, sA, sB)

        def body(j, mrow):
            z = zero_s[0]
            for u in range(A_NH):
                it = A_NH * j + (u + 1)
                if u % 2 == 0:
                    mrow = step_A(it, z, mrow, sB, sA)
                else:
                    mrow = step_A(it, z, mrow, sA, sB)
            return mrow

        return lax.fori_loop(0, (A_NIT - 2) // A_NH, body, m1)

    def proj_B(t):
        xn = xnB[t]
        yq = _dot(wbT[0:D, :], xn)
        q = _repitch(yq * QSCALE, H, one_fill).astype(BF16)
        for i in range(P_NB):
            qT[t * P_NB + i] = q[:, i * LB:(i + 1) * LB]
        yk = _dot(wbT[D:2 * D, :], xn)
        if isinstance(t, int):
            krows = pl.ds(2 * LB + t * P_TB, P_TB)
        else:
            krows = pl.ds(pl.multiple_of(2 * LB + t * P_TB, LB), P_TB)
        for h in range(H):
            kh = jnp.concatenate([yk[h * DH:(h + 1) * DH], zero_fill] * B_U, axis=0)
            kB[h, krows, :] = kh.T.astype(BF16)
        v = _repitch(_dot(wbT[2 * D:3 * D, :], xn), H, one_fill).astype(BF16)
        for i in range(P_NB):
            vTB[2 + t * P_NB + i] = v[:, i * LB:(i + 1) * LB]

    lane_p = _lane((B_SB, LB)) // B_SB

    def qk_B(b, s_ref, h, first=0):
        q = qT[b, h * DP:(h + 1) * DP, :]
        wq = jnp.concatenate(
            [_sel(lambda ln, u=u: ln // B_SB == u, q, None) for u in range(B_U)], axis=0)
        cols = slice(h * LB, (h + 1) * LB)

        def k_blk(i):
            if first:
                return kB[h, (b + i) * LB:(b + i + 1) * LB, :]
            return kB[h, pl.ds(pl.multiple_of((b + i) * LB, LB), LB), :]

        k_old, k_new = k_blk(0), k_blk(2)
        rows = [k_new[0:B_SB]]
        for rr in range(B_U - 1):
            rows.append(_sel(lambda ln, rr=rr: ln // DP <= rr,
                             k_old[rr * B_SB:(rr + 1) * B_SB],
                             k_new[(rr + 1) * B_SB:(rr + 2) * B_SB]))
        if not first:
            rows.append(k_old[(B_U - 1) * B_SB:])
        nr = len(rows) * B_SB
        s2 = _dot(jnp.concatenate(rows, axis=0), wq) + bias[0:nr, :]
        s_ref[0, LB:LB + nr, cols] = s2
        mm = jnp.max(s2.reshape(nr // 8, 8, LB), axis=0)
        if first != 1:
            s1 = _dot(k_blk(1), wq)
            s_ref[0, 0:LB, cols] = s1
            mm = jnp.maximum(mm, jnp.max(s1.reshape(LB // 8, 8, LB), axis=0))
        if first == 2:
            s_ref[0, 2 * LB:B_R, cols] = jnp.full((B_SB, LB), NEG, F32)
        return jnp.max(mm, axis=0, keepdims=True)

    def pv_B(b, z, s_ref, h, mrow, first=False):
        def ex(lo, hi):
            return jnp.exp2(s_ref[z, lo:hi, h * LB:(h + 1) * LB] - mrow)

        rows = slice(h * DP, (h + 1) * DP)
        news = [ex(LB, LB + B_SB)]
        olds = []
        for rr in range(B_U - 1):
            px = ex(LB + (rr + 1) * B_SB, LB + (rr + 2) * B_SB)
            olds.append(jnp.where(lane_p <= rr, px, 0.0))
            news.append(jnp.where(lane_p > rr, px, 0.0))
        acc = _dot(vTB[b + 2, rows, :], jnp.concatenate(news, axis=0).astype(BF16))
        if not first:
            olds.append(ex(2 * LB, B_R))
            acc = (acc + _dot(vTB[b + 1, rows, :], ex(0, LB).astype(BF16))
                   + _dot(vTB[b, rows, :], jnp.concatenate(olds, axis=0).astype(BF16)))
        oT[b, rows, :] = (acc * (1.0 / acc[DH:DH + 1, :])).astype(BF16)

    def step_B(b, z, mrows, s_cur, s_nxt, first=False):
        m = []
        for h in range(H + B_LEAD):
            if h < H:
                m.append(qk_B(b + 1, s_nxt, h, first=2 if first else 0))
            if h >= B_LEAD:
                pv_B(b, z, s_cur, h - B_LEAD, mrows[h - B_LEAD], first=first)
        return tuple(m)

    def attn_B_main():
        m0 = tuple(qk_B(0, sC, h, first=1) for h in range(H))
        m1 = step_B(0, zero_s[0], m0, sC, sD, first=True)

        def body(jj, mrows):
            z = zero_s[0]
            mrows = step_B(2 * jj + 1, z, mrows, sD, sC)
            return step_B(2 * jj + 2, z, mrows, sC, sD)

        return lax.fori_loop(0, (NB - 2) // 2, body, m1)

    def attn_B_last(mrows):
        z = zero_s[0]
        for h in range(H):
            pv_B(NB - 1, z, sD, h, mrows[h])

    zpad = jnp.zeros((DP - DH, D), F32)
    for cp in w_copies[:3]:
        cp.wait()
    waT[0:D, :] = wq_raw[...].T
    waT[D:D + 2 * DP, :] = jnp.concatenate(
        [wkT_raw[...].astype(F32), zpad, wvT_raw[...].astype(F32), zpad], axis=0).astype(BF16)
    for t in range(P_NT):
        x_copy(t).wait()
        store_x(t, x_raw[t].astype(F32))
    for cp in w_copies[3:]:
        cp.start()

    def out_copy(t):
        return pltpu.make_async_copy(out_stage.at[t], out_hbm.at[:, pl.ds(t * P_TB, P_TB)], osems.at[t])

    def rep(r_idx, carry):
        for b0, nb in A_PROJ_CHUNKS:
            proj_A(b0, nb)

        mA_last = attn_A_main()

        @pl.when(r_idx == 0)
        def _():
            for cp in w_copies[3:]:
                cp.wait()
            woAT[...] = _repitch(woA_raw[...].astype(F32), H, zpad).astype(BF16).T

        wbT[...] = wqkv_raw[...].T
        for t in range(P_NT):
            if t == LAST_POS:
                step_A(A_NIT - 1, zero_s[0], mA_last, sB, None, last=True)
            xs = out_proj(woAT, t)
            store_x(t, xs)
            xnB[t] = layernorm_T(xs)
        proj_B(0)

        def proj_B_body(t, c):
            proj_B(t)
            return c

        lax.fori_loop(1, P_NT, proj_B_body, 0)

        m_last = attn_B_main()

        @pl.when(r_idx == 1)
        def _():
            for t in range(P_NT):
                out_copy(t).wait()

        woBT[...] = _repitch(woB_raw[...].astype(F32), H, zpad).astype(BF16).T
        for t in range(P_NT):
            if t == LAST_POS_B:
                attn_B_last(m_last)
            xs = out_proj(woBT, t)
            store_x(t, xs)
            out_stage[t] = xs.astype(out_stage.dtype)
            out_copy(t).start()
        return carry

    lax.fori_loop(0, 2, rep, 0)
    for t in range(P_NT):
        out_copy(t).wait()


@jax.jit
def pallas_interleave_layers__grouped_kv_mqa__sliding_block__prompt_kernel(
    A_x: jax.Array,
    A_wq: jax.Array,
    A_wk: jax.Array,
    A_wv: jax.Array,
    A_wo: jax.Array,
    B_x: jax.Array,
    B_wqkv: jax.Array,
    B_wo: jax.Array,
):
    del B_x
    any_spec = pl.BlockSpec(memory_space=pl.ANY)
    outT = pl.pallas_call(
        _kernel,
        out_shape=jax.ShapeDtypeStruct((D, S), A_x.dtype),
        in_specs=[any_spec] * 7,
        out_specs=any_spec,
        scratch_shapes=[
            pltpu.VMEM((P_NT, D, P_TB), BF16),
            pltpu.VMEM((D, D), BF16),
            pltpu.VMEM((DH, D), BF16),
            pltpu.VMEM((DH, D), BF16),
            pltpu.VMEM((D, D), BF16),
            pltpu.VMEM((D, 3 * D), BF16),
            pltpu.VMEM((D, D), BF16),
            pltpu.VMEM((P_NT, D, P_TB), BF16),
            pltpu.VMEM((D + 2 * DP, D), BF16),
            pltpu.VMEM((D, HP), BF16),
            pltpu.VMEM((3 * D, D), BF16),
            pltpu.VMEM((D, HP), BF16),
            pltpu.VMEM((NB, D, LB), F32),
            pltpu.VMEM((P_NT, D, P_TB), BF16),
            pltpu.VMEM((NB, HP, LB), BF16),
            pltpu.VMEM((S, DP), BF16),
            pltpu.VMEM((DP, S), BF16),
            pltpu.VMEM((H, S + 2 * LB, LB), BF16),
            pltpu.VMEM((NB + 2, HP, LB), BF16),
            pltpu.VMEM((NB, HP, LB), BF16),
            pltpu.VMEM((1, S, A_TQ), F32),
            pltpu.VMEM((1, S, A_TQ), F32),
            pltpu.VMEM((1, B_R, H * LB), F32),
            pltpu.VMEM((1, B_R, H * LB), F32),
            pltpu.VMEM((B_RB, LB), F32),
            pltpu.SMEM((1,), jnp.int32),
            pltpu.SemaphoreType.DMA((P_NT + 6,)),
            pltpu.SemaphoreType.DMA((P_NT,)),
        ],
        compiler_params=pltpu.CompilerParams(vmem_limit_bytes=100 * 2**20),
    )(A_x[0].T, A_wq, A_wk.T, A_wv.T, A_wo, B_wqkv, B_wo)
    return outT.T[None]
```

```python
import functools

import jax
import jax.numpy as jnp
from jax import lax
import jax.experimental.pallas as pl
import jax.experimental.pallas.tpu as pltpu

S = 2048
D = 448
H = 16
DH = 28
DP = 32
HP = H * DP
DQ = DP // 2
W = 256
LB = 128
NB = S // LB
LH = LB // 2
EPS = 1e-5
NEG = -1e30
QSCALE = (DH ** -0.5) * 1.4426950408889634

A_TQ = 256
A_NC = S // LB
A_KV = 8 * A_NC
A_QB = [((S - A_KV) * c // A_NC) // 16 * 16 for c in range(A_NC + 1)]
A_LQ = 4
A_DELTA = 6
A_OFF = 6
A_SHIFT = 6
N_ZERO = 64
A_NQ = A_TQ // LB
A_NH = 18
A_NIT = (S // A_TQ) * H
P_TB = 512
P_NB = P_TB // LB
P_NT = S // P_TB
A_PROJ_CHUNKS = ((0, 1), (1, 3), (4, 4), (8, 4), (12, 4))

B_U = 4
B_SB = LB // B_U
B_RB = LB + B_SB
B_R = LB + B_RB
B_LEAD = 3

A_LAST_SPLIT = ((), range(0, 6), range(6, 12), range(12, 16))
B_LAST_SPLIT = (range(0, 4), range(4, 8), range(8, 12), range(12, 16))

F32 = jnp.float32
U32 = jnp.uint32
BF16 = jnp.bfloat16


def _dot(a, b):
    return jnp.dot(a, b, preferred_element_type=F32)


def _lane(shape):
    return lax.broadcasted_iota(jnp.int32, shape, 1)


def _sel(mask_fn, a, b):
    bu = jnp.zeros_like(a) if b is None else b
    return jnp.where(mask_fn(_lane(a.shape)), a, bu)


def _pk(x):
    return pltpu.bitcast(x, U32)


def _up(u):
    return pltpu.bitcast(u, BF16)


def _repitch(y, n_heads, fill):
    parts = []
    for h in range(n_heads):
        parts += [y[h * DH:(h + 1) * DH], fill]
    return jnp.concatenate(parts, axis=0)


def _kernel(xT_hbm, wq_hbm, wkT_hbm, wvT_hbm, woA_hbm, wqkv_hbm, woB_hbm, out_hbm,
            x_raw, wq_raw, wkT_raw, wvT_raw, woA_raw, wqkv_raw, woB_raw, out_stage,
            waT, woAT, wbT, woBT,
            xT, xnB, qT, kA, vTA, kB, vTB, oT, sA, sB, sv0, sv1, q32, kb, sC, sD, bias, zero_v, zero_s, sems, osems):
    for i in range(N_ZERO):
        zero_s[i] = 0
    zero_v[...] = jnp.zeros(zero_v.shape, U32)

    def x_copy(t):
        return pltpu.make_async_copy(xT_hbm.at[:, pl.ds(t * P_TB, P_TB)], x_raw.at[t], sems.at[t])

    w_copies = [
        pltpu.make_async_copy(src, dst, sems.at[P_NT + i])
        for i, (src, dst) in enumerate([
            (wq_hbm, wq_raw), (wkT_hbm, wkT_raw), (wvT_hbm, wvT_raw),
            (woA_hbm, woA_raw), (wqkv_hbm, wqkv_raw), (woB_hbm, woB_raw)])
    ]
    for cp in w_copies[:3]:
        cp.start()
    for t in range(P_NT):
        x_copy(t).start()

    r = lax.broadcasted_iota(jnp.int32, (B_RB, LB), 0)
    c = lax.broadcasted_iota(jnp.int32, (B_RB, LB), 1)
    use_new = (c // B_SB) >= (r // B_SB)
    ok = jnp.logical_or(jnp.logical_and(use_new, r <= c),
                        jnp.logical_and(jnp.logical_not(use_new), r - B_SB > c))
    bias[...] = jnp.where(ok, 0.0, NEG).astype(F32)
    null_k = jnp.where(_lane((2 * LB, LB)) % DP == DH, NEG, 0.0).astype(BF16)
    for h in range(H):
        kB[h, 0:LB, :] = _pk(null_k)
    vTB[0:2] = jnp.zeros((2, HP // 2, LB), U32)

    def fills(n):
        return (jnp.zeros((DP - DH, n), F32),
                (lax.broadcasted_iota(jnp.int32, (DP - DH, n), 0) == 0).astype(F32))

    zero_fill, one_fill = fills(P_TB)

    def load_x(t):
        return jnp.concatenate([xT[t * P_NB + i] for i in range(P_NB)], axis=1)

    def store_x(t, xs):
        for i in range(P_NB):
            xT[t * P_NB + i] = xs[:, i * LB:(i + 1) * LB]

    def colsum(a):
        if a.shape[1] > LB:
            return jnp.sum(a, axis=0, keepdims=True)
        parts = [a[i * 8:(i + 1) * 8] for i in range(a.shape[0] // 8)]
        while len(parts) > 1:
            parts = ([parts[i] + parts[i + 1] for i in range(0, len(parts) - 1, 2)]
                     + ([parts[-1]] if len(parts) % 2 else []))
        return jnp.sum(parts[0], axis=0, keepdims=True)

    def layernorm_T(xs):
        m = colsum(xs) * (1.0 / D)
        xc = xs - m
        v = colsum(xc * xc) * (1.0 / D)
        return (xc * lax.rsqrt(v + EPS)).astype(BF16)

    def out_proj(wo_ref, t):
        o = _up(jnp.concatenate([oT[t * P_NB + i] for i in range(P_NB)], axis=1))
        return load_x(t) + _dot(_up(wo_ref[...]), o)

    def proj_A(b0, nb):
        n = nb * LB
        zf, of = fills(n)
        xn = layernorm_T(jnp.concatenate([xT[b0 + i] for i in range(nb)], axis=1))
        y = _dot(_up(waT[...]), xn)
        qf = _repitch(y[:D] * QSCALE, H, zf)
        q = _pk(qf.astype(BF16))
        for i in range(nb):
            qT[b0 + i] = q[:, i * LB:(i + 1) * LB]
            bb = b0 + i
            q32[(bb // A_NQ) * H:(bb // A_NQ + 1) * H, :, (bb % A_NQ) * LB:(bb % A_NQ + 1) * LB] = (
                qf[:, i * LB:(i + 1) * LB].reshape(H, DP, LB))
        kA[b0 * LB // 2:(b0 * LB + n) // 2, :] = _pk(y[D:D + DP].T.astype(BF16))
        if b0 == 0:
            for d in range(DH):
                kb[d] = jnp.broadcast_to(y[D + d:D + d + 1, 0:A_KV], (LB, A_KV)).T
        v = _repitch(y[D + DP:D + DP + DH], 1, of)
        vTA[:, b0 * LB:b0 * LB + n] = _pk(v.astype(BF16))

    neg_A = jnp.full((8, A_TQ), -jnp.inf, F32)
    svs = (sv0, sv1)

    def zero_of(x, z):
        return lax.bitcast_convert_type(x, U32) & zero_v[z]

    def qk_chunk(qu, s_ref, ci, m):
        lo, hi = A_QB[ci], A_QB[ci + 1]
        s = _dot(_up(kA[(A_KV + lo) // 2:(A_KV + hi) // 2, :]), _up(qu))
        s_ref[0, lo:hi, :] = s
        mm = jnp.max(s.reshape((hi - lo) // 8, 8, A_TQ), axis=0)
        return jnp.maximum(m, mm), mm

    def qk_head_mxu(it):
        s = _dot(_up(kA[0:A_KV // 2, :]), _up(q_blk(it)))
        svs[it % 2][0] = s
        return jnp.max(s.reshape(A_KV // 8, 8, A_TQ), axis=0)

    def qk_piece(it, zi, sv_ref, p, rel, z):
        qi = it + zero_s[zi]
        accs = [None] * A_NQ
        if rel is not None:
            zz = lax.bitcast_convert_type(zero_of(rel, z), F32)
            accs = [zz[:, l * LB:(l + 1) * LB] for l in range(A_NQ)]
        for d in range(DH):
            kd = kb[d, p * 8:(p + 1) * 8, :]
            for l in range(A_NQ):
                t = kd * q32[qi, d:d + 1, l * LB:(l + 1) * LB]
                accs[l] = t if accs[l] is None else accs[l] + t
        s = jnp.concatenate(accs, axis=1)
        sv_ref[0, p * 8:(p + 1) * 8, :] = s
        return s

    def pv_chunk(s_ref, sv_ref, z, ci, mrow, acc):
        s = sv_ref[z] if ci == 0 else s_ref[z, (ci - 1) * LB:ci * LB, :]
        p = jnp.exp2(s - mrow).astype(BF16)
        return acc + _dot(_up(vTA[:, ci * LB:(ci + 1) * LB]), p)

    def a_index(it):
        if isinstance(it, int):
            return (it // H) * A_NQ, it % H
        return lax.shift_right_logical(it, 4) * A_NQ, it & (H - 1)

    def a_rows(h):
        return pl.ds(h * DQ if isinstance(h, int) else pl.multiple_of(h * DQ, DQ), DQ)

    def q_blk(it):
        qb, h = a_index(it)
        return jnp.concatenate([qT[qb + i, a_rows(h), :] for i in range(A_NQ)], axis=1)

    def finish_A(it, acc):
        qb, h = a_index(it)
        o = _pk((acc * (1.0 / acc[DH:DH + 1, :])).astype(BF16))
        for i in range(A_NQ):
            oT[qb + i, a_rows(h), :] = o[:, i * LB:(i + 1) * LB]

    def steps_A(it0, par, n_steps, m8, mv_acc, first_piece):
        z = zero_s[0]
        gates = {}

        def run_piece(r, rel):
            if not (first_piece <= r < n_steps * A_NC - A_SHIFT):
                return
            n = r + 2 * A_NC - A_OFF
            blk, p = n // A_NC, n % A_NC
            it = it0 + blk
            it = min(it, A_NIT - 1) if isinstance(it, int) else jnp.minimum(it, A_NIT - 1)
            x = qk_piece(it, 1 + n % (N_ZERO - 1), svs[(par + blk) % 2], p, rel, z)
            mv_acc[blk] = x if blk not in mv_acc else jnp.maximum(mv_acc[blk], x)
            gates[r] = x

        for r in range(-A_SHIFT, 0):
            run_piece(r, None)
        for u in range(n_steps):
            it = it0 + u
            s_cur, s_nxt = (sA, sB) if (par + u) % 2 == 0 else (sB, sA)
            sv_cur = svs[(par + u) % 2]
            mrow = jnp.max(m8, axis=0, keepdims=True)
            qn = q_blk(it + 1)
            m = neg_A
            acc = jnp.zeros((DP, A_TQ), F32)
            for c in range(A_NC + A_LQ):
                if c < A_NC:
                    g = u * A_NC + c
                    qu = qn
                    if (g - A_DELTA) in gates:
                        qu = jnp.concatenate(
                            [qn[0:8] | zero_of(gates[g - A_DELTA], z), qn[8:DQ]], axis=0)
                    m, mm = qk_chunk(qu, s_nxt, c, m)
                    run_piece(g, mm)
                if c >= A_LQ:
                    acc = pv_chunk(s_cur, sv_cur, z, c - A_LQ, mrow, acc)
            finish_A(it, acc)
            m8 = jnp.maximum(m, mv_acc[u + 1])
        return m8, mv_acc[n_steps + 1]

    def attn_A_main():
        q0 = q_blk(0)
        m = qk_head_mxu(0)
        for ci in range(A_NC):
            m, _ = qk_chunk(q0, sA, ci, m)
        carry = steps_A(0, 0, 1, m, {1: qk_head_mxu(1)}, A_OFF)

        def body(j, carry):
            return steps_A(A_NH * j + 1, 1, A_NH, carry[0], {1: carry[1]}, -A_SHIFT)

        m_last, _ = lax.fori_loop(0, (A_NIT - 2) // A_NH, body, carry)
        return jnp.max(m_last, axis=0, keepdims=True)

    def proj_B(t):
        xn = xnB[t]
        yq = _dot(_up(wbT[0:D // 2, :]), xn)
        q = _pk(_repitch(yq * QSCALE, H, one_fill).astype(BF16))
        for i in range(P_NB):
            qT[t * P_NB + i] = q[:, i * LB:(i + 1) * LB]
        yk = _dot(_up(wbT[D // 2:D, :]), xn)
        if isinstance(t, int):
            krows = pl.ds(LB + t * (P_TB // 2), P_TB // 2)
        else:
            krows = pl.ds(pl.multiple_of(LB + t * (P_TB // 2), LB), P_TB // 2)
        for h in range(H):
            kh = jnp.concatenate([yk[h * DH:(h + 1) * DH], zero_fill] * B_U, axis=0)
            kB[h, krows, :] = _pk(kh.T.astype(BF16))
        v = _pk(_repitch(_dot(_up(wbT[D:3 * D // 2, :]), xn), H, one_fill).astype(BF16))
        for i in range(P_NB):
            vTB[2 + t * P_NB + i] = v[:, i * LB:(i + 1) * LB]

    lane_p = _lane((B_SB, LB)) // B_SB

    def qk_B(b, s_ref, h, first=0):
        q = qT[b, h * DQ:(h + 1) * DQ, :]
        wq = _up(jnp.concatenate(
            [_sel(lambda ln, u=u: ln // B_SB == u, q, None) for u in range(B_U)], axis=0))
        cols = slice(h * LB, (h + 1) * LB)

        def k_blk(i):
            if first:
                return kB[h, (b + i) * LH:(b + i + 1) * LH, :]
            return kB[h, pl.ds(pl.multiple_of((b + i) * LH, LH), LH), :]

        k_old, k_new = k_blk(0), k_blk(2)
        sh = B_SB // 2
        rows = [k_new[0:sh]]
        for rr in range(B_U - 1):
            rows.append(_sel(lambda ln, rr=rr: ln // DP <= rr,
                             k_old[rr * sh:(rr + 1) * sh], k_new[(rr + 1) * sh:(rr + 2) * sh]))
        if not first:
            rows.append(k_old[(B_U - 1) * sh:])
        nr = len(rows) * B_SB
        s2 = _dot(_up(jnp.concatenate(rows, axis=0)), wq) + bias[0:nr, :]
        s_ref[0, LB:LB + nr, cols] = s2
        mm = jnp.max(s2.reshape(nr // 8, 8, LB), axis=0)
        if first != 1:
            s1 = _dot(_up(k_blk(1)), wq)
            s_ref[0, 0:LB, cols] = s1
            mm = jnp.maximum(mm, jnp.max(s1.reshape(LB // 8, 8, LB), axis=0))
        if first == 2:
            s_ref[0, 2 * LB:B_R, cols] = jnp.full((B_SB, LB), NEG, F32)
        return jnp.max(mm, axis=0, keepdims=True)

    def pv_B(b, z, s_ref, h, mrow, first=False):
        def ex(lo, hi):
            return jnp.exp2(s_ref[z, lo:hi, h * LB:(h + 1) * LB] - mrow)

        rows = slice(h * DQ, (h + 1) * DQ)
        news = [ex(LB, LB + B_SB)]
        olds = []
        for rr in range(B_U - 1):
            px = ex(LB + (rr + 1) * B_SB, LB + (rr + 2) * B_SB)
            olds.append(jnp.where(lane_p <= rr, px, 0.0))
            news.append(jnp.where(lane_p > rr, px, 0.0))
        acc = _dot(_up(vTB[b + 2, rows, :]), jnp.concatenate(news, axis=0).astype(BF16))
        if not first:
            olds.append(ex(2 * LB, B_R))
            acc = (acc + _dot(_up(vTB[b + 1, rows, :]), ex(0, LB).astype(BF16))
                   + _dot(_up(vTB[b, rows, :]), jnp.concatenate(olds, axis=0).astype(BF16)))
        oT[b, rows, :] = _pk((acc * (1.0 / acc[DH:DH + 1, :])).astype(BF16))

    def step_B(b, z, mrows, s_cur, s_nxt, first=False):
        m = []
        for h in range(H + B_LEAD):
            if h < H:
                m.append(qk_B(b + 1, s_nxt, h, first=2 if first else 0))
            if h >= B_LEAD:
                pv_B(b, z, s_cur, h - B_LEAD, mrows[h - B_LEAD], first=first)
        return tuple(m)

    def attn_B_main():
        m0 = tuple(qk_B(0, sC, h, first=1) for h in range(H))
        m1 = step_B(0, zero_s[0], m0, sC, sD, first=True)

        def body(jj, mrows):
            z = zero_s[0]
            mrows = step_B(2 * jj + 1, z, mrows, sD, sC)
            return step_B(2 * jj + 2, z, mrows, sC, sD)

        return lax.fori_loop(0, (NB - 2) // 2, body, m1)

    zpad = jnp.zeros((DP - DH, D), F32)
    for cp in w_copies[:3]:
        cp.wait()
    waT[0:D // 2, :] = _pk(wq_raw[...].T)
    waT[D // 2:D // 2 + DP, :] = _pk(jnp.concatenate(
        [wkT_raw[...].astype(F32), zpad, wvT_raw[...].astype(F32), zpad], axis=0).astype(BF16))
    for t in range(P_NT):
        x_copy(t).wait()
        store_x(t, x_raw[t].astype(F32))
    for cp in w_copies[3:]:
        cp.start()

    def out_copy(t):
        return pltpu.make_async_copy(out_stage.at[t], out_hbm.at[:, pl.ds(t * P_TB, P_TB)], osems.at[t])

    def rep(r_idx, carry):
        for b0, nb in A_PROJ_CHUNKS:
            proj_A(b0, nb)

        mA_last = attn_A_main()

        @pl.when(r_idx == 0)
        def _():
            for cp in w_copies[3:]:
                cp.wait()
            woAT[...] = _pk(_repitch(woA_raw[...].astype(F32), H, zpad).astype(BF16).T)

        wbT[...] = _pk(wqkv_raw[...].T)
        zl = zero_s[0]
        acc = jnp.zeros((DP, A_TQ), F32)
        for t in range(P_NT):
            for ci in A_LAST_SPLIT[t]:
                acc = pv_chunk(sB, sv1, zl, ci, mA_last, acc)
            if t == P_NT - 1:
                finish_A(A_NIT - 1, acc)
            store_x(t, out_proj(woAT, t))
        for t in range(P_NT):
            xnB[t] = layernorm_T(load_x(t))
        proj_B(0)

        def proj_B_body(t, c):
            proj_B(t)
            return c

        lax.fori_loop(1, P_NT, proj_B_body, 0)

        m_last = attn_B_main()

        @pl.when(r_idx == 1)
        def _():
            for t in range(P_NT):
                out_copy(t).wait()

        woBT[...] = _pk(_repitch(woB_raw[...].astype(F32), H, zpad).astype(BF16).T)
        zl = zero_s[0]
        for t in range(P_NT):
            for h in B_LAST_SPLIT[t]:
                pv_B(NB - 1, zl, sD, h, m_last[h])
            xs = out_proj(woBT, t)
            store_x(t, xs)
            out_stage[t] = xs.astype(out_stage.dtype)
            out_copy(t).start()
        return carry

    lax.fori_loop(0, 2, rep, 0)
    for t in range(P_NT):
        out_copy(t).wait()


@jax.jit
def pallas_interleave_layers__grouped_kv_mqa__sliding_block__prompt_kernel(
    A_x: jax.Array,
    A_wq: jax.Array,
    A_wk: jax.Array,
    A_wv: jax.Array,
    A_wo: jax.Array,
    B_x: jax.Array,
    B_wqkv: jax.Array,
    B_wo: jax.Array,
):
    del B_x
    any_spec = pl.BlockSpec(memory_space=pl.ANY)
    outT = pl.pallas_call(
        _kernel,
        out_shape=jax.ShapeDtypeStruct((D, S), A_x.dtype),
        in_specs=[any_spec] * 7,
        out_specs=any_spec,
        scratch_shapes=[
            pltpu.VMEM((P_NT, D, P_TB), BF16),
            pltpu.VMEM((D, D), BF16),
            pltpu.VMEM((DH, D), BF16),
            pltpu.VMEM((DH, D), BF16),
            pltpu.VMEM((D, D), BF16),
            pltpu.VMEM((D, 3 * D), BF16),
            pltpu.VMEM((D, D), BF16),
            pltpu.VMEM((P_NT, D, P_TB), BF16),
            pltpu.VMEM((D // 2 + DP, D), U32),
            pltpu.VMEM((D // 2, HP), U32),
            pltpu.VMEM((3 * D // 2, D), U32),
            pltpu.VMEM((D // 2, HP), U32),
            pltpu.VMEM((NB, D, LB), F32),
            pltpu.VMEM((P_NT, D, P_TB), BF16),
            pltpu.VMEM((NB, HP // 2, LB), U32),
            pltpu.VMEM((S // 2, DP), U32),
            pltpu.VMEM((DQ, S), U32),
            pltpu.VMEM((H, S // 2 + LB, LB), U32),
            pltpu.VMEM((NB + 2, HP // 2, LB), U32),
            pltpu.VMEM((NB, HP // 2, LB), U32),
            pltpu.VMEM((1, S - A_KV, A_TQ), F32),
            pltpu.VMEM((1, S - A_KV, A_TQ), F32),
            pltpu.VMEM((1, A_KV, A_TQ), F32),
            pltpu.VMEM((1, A_KV, A_TQ), F32),
            pltpu.VMEM((A_NIT, DP, A_TQ), F32),
            pltpu.VMEM((DH, A_KV, LB), F32),
            pltpu.VMEM((1, B_R, H * LB), F32),
            pltpu.VMEM((1, B_R, H * LB), F32),
            pltpu.VMEM((B_RB, LB), F32),
            pltpu.VMEM((1, 8, A_TQ), U32),
            pltpu.SMEM((N_ZERO,), jnp.int32),
            pltpu.SemaphoreType.DMA((P_NT + 6,)),
            pltpu.SemaphoreType.DMA((P_NT,)),
        ],
        compiler_params=pltpu.CompilerParams(vmem_limit_bytes=100 * 2**20),
    )(A_x[0].T, A_wq, A_wk.T, A_wv.T, A_wo, B_wqkv, B_wo)
    return outT.T[None]
```

```python
import functools

import jax
import jax.numpy as jnp
from jax import lax
import jax.experimental.pallas as pl
import jax.experimental.pallas.tpu as pltpu

S = 2048
D = 448
H = 16
DH = 28
DP = 32
HP = H * DP
DQ = DP // 2
W = 256
LB = 128
NB = S // LB
LH = LB // 2
EPS = 1e-5
NEG = -1e30
QSCALE = (DH ** -0.5) * 1.4426950408889634

A_TQ = 256
A_NC = S // LB
A_KV = 8 * A_NC
A_QB = [((S - A_KV) * c // A_NC) // 16 * 16 for c in range(A_NC + 1)]
A_LQ = 3
A_DELTA = 5
A_OFF = 6
A_SHIFT = 6
N_ZERO = 64
A_NQ = A_TQ // LB
A_NH = 18
A_NIT = (S // A_TQ) * H
P_TB = 512
P_NB = P_TB // LB
P_NT = S // P_TB
A_PROJ_CHUNKS = ((0, 1), (1, 3), (4, 4), (8, 4), (12, 4))

B_U = 4
B_SB = LB // B_U
B_RB = LB + B_SB
B_R = LB + B_RB
B_LEAD = 3

A_LAST_SPLIT = ((), range(0, 6), range(6, 12), range(12, 16))
OUT_CHUNKS = ((0, 4), (4, 4), (8, 4), (12, 2), (14, 2))
B_LAST_SPLIT = (range(0, 4), range(4, 8), range(8, 12), range(12, 16), ())

F32 = jnp.float32
U32 = jnp.uint32
BF16 = jnp.bfloat16


def _dot(a, b):
    return jnp.dot(a, b, preferred_element_type=F32)


def _lane(shape):
    return lax.broadcasted_iota(jnp.int32, shape, 1)


def _sel(mask_fn, a, b):
    bu = jnp.zeros_like(a) if b is None else b
    return jnp.where(mask_fn(_lane(a.shape)), a, bu)


def _pk(x):
    return pltpu.bitcast(x, U32)


def _up(u):
    return pltpu.bitcast(u, BF16)


def _repitch(y, n_heads, fill):
    parts = []
    for h in range(n_heads):
        parts += [y[h * DH:(h + 1) * DH], fill]
    return jnp.concatenate(parts, axis=0)


def _kernel(xT_hbm, wq_hbm, wkT_hbm, wvT_hbm, woA_hbm, wqkv_hbm, woB_hbm, out_hbm,
            x_raw, wq_raw, wkT_raw, wvT_raw, woA_raw, wqkv_raw, woB_raw, out_stage,
            waT, woAT, wbT, woBT,
            xT, xnB, qT, kA, vTA, kB, vTB, oT, sA, sB, sv0, sv1, q32, kb, sC, sD, bias, zero_v, zero_s, sems, osems):
    def x_copy(t):
        return pltpu.make_async_copy(xT_hbm.at[:, pl.ds(t * P_TB, P_TB)], x_raw.at[t], sems.at[t])

    w_copies = [
        pltpu.make_async_copy(src, dst, sems.at[P_NT + i])
        for i, (src, dst) in enumerate([
            (wq_hbm, wq_raw), (wkT_hbm, wkT_raw), (wvT_hbm, wvT_raw),
            (woA_hbm, woA_raw), (wqkv_hbm, wqkv_raw), (woB_hbm, woB_raw)])
    ]
    for cp in w_copies[:3]:
        cp.start()
    for t in range(P_NT):
        x_copy(t).start()

    for i in range(N_ZERO):
        zero_s[i] = 0
    zero_v[...] = jnp.zeros(zero_v.shape, U32)

    r = lax.broadcasted_iota(jnp.int32, (B_RB, LB), 0)
    c = lax.broadcasted_iota(jnp.int32, (B_RB, LB), 1)
    use_new = (c // B_SB) >= (r // B_SB)
    ok = jnp.logical_or(jnp.logical_and(use_new, r <= c),
                        jnp.logical_and(jnp.logical_not(use_new), r - B_SB > c))
    bias[...] = jnp.where(ok, 0.0, NEG).astype(F32)
    null_k = jnp.where(_lane((2 * LB, LB)) % DP == DH, NEG, 0.0).astype(BF16)
    for h in range(H):
        kB[h, 0:LB, :] = _pk(null_k)
    vTB[0:2] = jnp.zeros((2, HP // 2, LB), U32)

    def fills(n):
        return (jnp.zeros((DP - DH, n), F32),
                (lax.broadcasted_iota(jnp.int32, (DP - DH, n), 0) == 0).astype(F32))

    zero_fill, one_fill = fills(P_TB)

    def load_x(t):
        return jnp.concatenate([xT[t * P_NB + i] for i in range(P_NB)], axis=1)

    def store_x(t, xs):
        for i in range(P_NB):
            xT[t * P_NB + i] = xs[:, i * LB:(i + 1) * LB]

    def colsum(a):
        if a.shape[1] > LB:
            return jnp.sum(a, axis=0, keepdims=True)
        parts = [a[i * 8:(i + 1) * 8] for i in range(a.shape[0] // 8)]
        while len(parts) > 1:
            parts = ([parts[i] + parts[i + 1] for i in range(0, len(parts) - 1, 2)]
                     + ([parts[-1]] if len(parts) % 2 else []))
        return jnp.sum(parts[0], axis=0, keepdims=True)

    def layernorm_T(xs):
        m = colsum(xs) * (1.0 / D)
        xc = xs - m
        v = colsum(xc * xc) * (1.0 / D)
        return (xc * lax.rsqrt(v + EPS)).astype(BF16)

    def out_proj(wo_ref, t):
        o = _up(jnp.concatenate([oT[t * P_NB + i] for i in range(P_NB)], axis=1))
        return load_x(t) + _dot(_up(wo_ref[...]), o)

    def proj_A(b0, nb):
        n = nb * LB
        zf, of = fills(n)
        xn = layernorm_T(jnp.concatenate([xT[b0 + i] for i in range(nb)], axis=1))
        y = _dot(_up(waT[...]), xn)
        qf = _repitch(y[:D] * QSCALE, H, zf)
        q = _pk(qf.astype(BF16))
        for i in range(nb):
            qT[b0 + i] = q[:, i * LB:(i + 1) * LB]
            bb = b0 + i
            q32[(bb // A_NQ) * H:(bb // A_NQ + 1) * H, :, (bb % A_NQ) * LB:(bb % A_NQ + 1) * LB] = (
                qf[:, i * LB:(i + 1) * LB].reshape(H, DP, LB))
        kA[b0 * LB // 2:(b0 * LB + n) // 2, :] = _pk(y[D:D + DP].T.astype(BF16))
        if b0 == 0:
            for d in range(DH):
                kb[d] = jnp.broadcast_to(y[D + d:D + d + 1, 0:A_KV], (LB, A_KV)).T
        v = _repitch(y[D + DP:D + DP + DH], 1, of)
        vTA[:, b0 * LB:b0 * LB + n] = _pk(v.astype(BF16))

    neg_A = jnp.full((8, A_TQ), -jnp.inf, F32)
    svs = (sv0, sv1)

    def zero_of(x, z):
        return lax.bitcast_convert_type(x, U32) & zero_v[z]

    def qk_chunk(qu, s_ref, ci, m):
        lo, hi = A_QB[ci], A_QB[ci + 1]
        s = _dot(_up(kA[(A_KV + lo) // 2:(A_KV + hi) // 2, :]), _up(qu))
        s_ref[0, lo:hi, :] = s
        mm = jnp.max(s.reshape((hi - lo) // 8, 8, A_TQ), axis=0)
        return jnp.maximum(m, mm), mm

    def qk_head_mxu(it):
        s = _dot(_up(kA[0:A_KV // 2, :]), _up(q_blk(it)))
        svs[it % 2][0] = s
        return jnp.max(s.reshape(A_KV // 8, 8, A_TQ), axis=0)

    def qk_piece(it, zi, sv_ref, p, rel, z):
        qi = it + zero_s[zi]
        accs = [None] * A_NQ
        if rel is not None:
            zz = lax.bitcast_convert_type(zero_of(rel, z), F32)
            accs = [zz[:, l * LB:(l + 1) * LB] for l in range(A_NQ)]
        for d in range(DH):
            kd = kb[d, p * 8:(p + 1) * 8, :]
            for l in range(A_NQ):
                t = kd * q32[qi, d:d + 1, l * LB:(l + 1) * LB]
                accs[l] = t if accs[l] is None else accs[l] + t
        s = jnp.concatenate(accs, axis=1)
        sv_ref[0, p * 8:(p + 1) * 8, :] = s
        return s

    def pv_chunk(s_ref, sv_ref, z, ci, mrow, acc):
        s = sv_ref[z] if ci == 0 else s_ref[z, (ci - 1) * LB:ci * LB, :]
        p = jnp.exp2(s - mrow).astype(BF16)
        return acc + _dot(_up(vTA[:, ci * LB:(ci + 1) * LB]), p)

    def a_index(it):
        if isinstance(it, int):
            return (it // H) * A_NQ, it % H
        return lax.shift_right_logical(it, 4) * A_NQ, it & (H - 1)

    def a_rows(h):
        return pl.ds(h * DQ if isinstance(h, int) else pl.multiple_of(h * DQ, DQ), DQ)

    def q_blk(it):
        qb, h = a_index(it)
        return jnp.concatenate([qT[qb + i, a_rows(h), :] for i in range(A_NQ)], axis=1)

    def finish_A(it, acc):
        qb, h = a_index(it)
        o = _pk((acc * (1.0 / acc[DH:DH + 1, :])).astype(BF16))
        for i in range(A_NQ):
            oT[qb + i, a_rows(h), :] = o[:, i * LB:(i + 1) * LB]

    def steps_A(it0, par, n_steps, m8, mv_acc, first_piece):
        z = zero_s[0]
        gates = {}

        def run_piece(r, rel):
            if not (first_piece <= r < n_steps * A_NC - A_SHIFT):
                return
            n = r + 2 * A_NC - A_OFF
            blk, p = n // A_NC, n % A_NC
            it = it0 + blk
            it = min(it, A_NIT - 1) if isinstance(it, int) else jnp.minimum(it, A_NIT - 1)
            x = qk_piece(it, 1 + n % (N_ZERO - 1), svs[(par + blk) % 2], p, rel, z)
            mv_acc[blk] = x if blk not in mv_acc else jnp.maximum(mv_acc[blk], x)
            gates[r] = x

        for r in range(-A_SHIFT, 0):
            run_piece(r, None)
        for u in range(n_steps):
            it = it0 + u
            s_cur, s_nxt = (sA, sB) if (par + u) % 2 == 0 else (sB, sA)
            sv_cur = svs[(par + u) % 2]
            mrow = jnp.max(m8, axis=0, keepdims=True)
            qn = q_blk(it + 1)
            m = neg_A
            acc = jnp.zeros((DP, A_TQ), F32)
            for c in range(A_NC + A_LQ):
                if c < A_NC:
                    g = u * A_NC + c
                    qu = qn
                    if (g - A_DELTA) in gates:
                        qu = jnp.concatenate(
                            [qn[0:8] | zero_of(gates[g - A_DELTA], z), qn[8:DQ]], axis=0)
                    m, mm = qk_chunk(qu, s_nxt, c, m)
                    run_piece(g, mm)
                if c >= A_LQ:
                    acc = pv_chunk(s_cur, sv_cur, z, c - A_LQ, mrow, acc)
            finish_A(it, acc)
            m8 = jnp.maximum(m, mv_acc[u + 1])
        return m8, mv_acc[n_steps + 1]

    def attn_A_main():
        q0 = q_blk(0)
        m = qk_head_mxu(0)
        for ci in range(A_NC):
            m, _ = qk_chunk(q0, sA, ci, m)
        carry = steps_A(0, 0, 1, m, {1: qk_head_mxu(1)}, A_OFF)

        def body(j, carry):
            return steps_A(A_NH * j + 1, 1, A_NH, carry[0], {1: carry[1]}, -A_SHIFT)

        m_last, _ = lax.fori_loop(0, (A_NIT - 2) // A_NH, body, carry)
        return jnp.max(m_last, axis=0, keepdims=True)

    def proj_B(t):
        xn = xnB[t]
        yq = _dot(_up(wbT[0:D // 2, :]), xn)
        q = _pk(_repitch(yq * QSCALE, H, one_fill).astype(BF16))
        for i in range(P_NB):
            qT[t * P_NB + i] = q[:, i * LB:(i + 1) * LB]
        yk = _dot(_up(wbT[D // 2:D, :]), xn)
        if isinstance(t, int):
            krows = pl.ds(LB + t * (P_TB // 2), P_TB // 2)
        else:
            krows = pl.ds(pl.multiple_of(LB + t * (P_TB // 2), LB), P_TB // 2)
        for h in range(H):
            kh = jnp.concatenate([yk[h * DH:(h + 1) * DH], zero_fill] * B_U, axis=0)
            kB[h, krows, :] = _pk(kh.T.astype(BF16))
        v = _pk(_repitch(_dot(_up(wbT[D:3 * D // 2, :]), xn), H, one_fill).astype(BF16))
        for i in range(P_NB):
            vTB[2 + t * P_NB + i] = v[:, i * LB:(i + 1) * LB]

    lane_p = _lane((B_SB, LB)) // B_SB

    def qk_B(b, s_ref, h, first=0):
        q = qT[b, h * DQ:(h + 1) * DQ, :]
        wq = _up(jnp.concatenate(
            [_sel(lambda ln, u=u: ln // B_SB == u, q, None) for u in range(B_U)], axis=0))
        cols = slice(h * LB, (h + 1) * LB)

        def k_blk(i):
            if first:
                return kB[h, (b + i) * LH:(b + i + 1) * LH, :]
            return kB[h, pl.ds(pl.multiple_of((b + i) * LH, LH), LH), :]

        k_old, k_new = k_blk(0), k_blk(2)
        sh = B_SB // 2
        rows = [k_new[0:sh]]
        for rr in range(B_U - 1):
            rows.append(_sel(lambda ln, rr=rr: ln // DP <= rr,
                             k_old[rr * sh:(rr + 1) * sh], k_new[(rr + 1) * sh:(rr + 2) * sh]))
        if not first:
            rows.append(k_old[(B_U - 1) * sh:])
        nr = len(rows) * B_SB
        s2 = _dot(_up(jnp.concatenate(rows, axis=0)), wq) + bias[0:nr, :]
        s_ref[0, LB:LB + nr, cols] = s2
        mm = jnp.max(s2.reshape(nr // 8, 8, LB), axis=0)
        if first != 1:
            s1 = _dot(_up(k_blk(1)), wq)
            s_ref[0, 0:LB, cols] = s1
            mm = jnp.maximum(mm, jnp.max(s1.reshape(LB // 8, 8, LB), axis=0))
        if first == 2:
            s_ref[0, 2 * LB:B_R, cols] = jnp.full((B_SB, LB), NEG, F32)
        return jnp.max(mm, axis=0, keepdims=True)

    def pv_B(b, z, s_ref, h, mrow, first=False):
        def ex(lo, hi):
            return jnp.exp2(s_ref[z, lo:hi, h * LB:(h + 1) * LB] - mrow)

        rows = slice(h * DQ, (h + 1) * DQ)
        news = [ex(LB, LB + B_SB)]
        olds = []
        for rr in range(B_U - 1):
            px = ex(LB + (rr + 1) * B_SB, LB + (rr + 2) * B_SB)
            olds.append(jnp.where(lane_p <= rr, px, 0.0))
            news.append(jnp.where(lane_p > rr, px, 0.0))
        acc = _dot(_up(vTB[b + 2, rows, :]), jnp.concatenate(news, axis=0).astype(BF16))
        if not first:
            olds.append(ex(2 * LB, B_R))
            acc = (acc + _dot(_up(vTB[b + 1, rows, :]), ex(0, LB).astype(BF16))
                   + _dot(_up(vTB[b, rows, :]), jnp.concatenate(olds, axis=0).astype(BF16)))
        oT[b, rows, :] = _pk((acc * (1.0 / acc[DH:DH + 1, :])).astype(BF16))

    def step_B(b, z, mrows, s_cur, s_nxt, first=False):
        m = []
        for h in range(H + B_LEAD):
            if h < H:
                m.append(qk_B(b + 1, s_nxt, h, first=2 if first else 0))
            if h >= B_LEAD:
                pv_B(b, z, s_cur, h - B_LEAD, mrows[h - B_LEAD], first=first)
        return tuple(m)

    def attn_B_main():
        m0 = tuple(qk_B(0, sC, h, first=1) for h in range(H))
        m1 = step_B(0, zero_s[0], m0, sC, sD, first=True)

        def body(jj, mrows):
            z = zero_s[0]
            mrows = step_B(2 * jj + 1, z, mrows, sD, sC)
            return step_B(2 * jj + 2, z, mrows, sC, sD)

        return lax.fori_loop(0, (NB - 2) // 2, body, m1)

    zpad = jnp.zeros((DP - DH, D), F32)
    for cp in w_copies[:3]:
        cp.wait()
    waT[0:D // 2, :] = _pk(wq_raw[...].T)
    waT[D // 2:D // 2 + DP, :] = _pk(jnp.concatenate(
        [wkT_raw[...].astype(F32), zpad, wvT_raw[...].astype(F32), zpad], axis=0).astype(BF16))
    for t in range(P_NT):
        x_copy(t).wait()
        store_x(t, x_raw[t].astype(F32))
    for cp in w_copies[3:]:
        cp.start()

    def out_copy(i):
        cols = pl.ds(OUT_CHUNKS[i][0] * LB, OUT_CHUNKS[i][1] * LB)
        return pltpu.make_async_copy(out_stage.at[:, cols], out_hbm.at[:, cols], osems.at[i])

    def rep(r_idx, carry):
        for b0, nb in A_PROJ_CHUNKS:
            proj_A(b0, nb)

        mA_last = attn_A_main()

        @pl.when(r_idx == 0)
        def _():
            for cp in w_copies[3:]:
                cp.wait()
            woAT[...] = _pk(_repitch(woA_raw[...].astype(F32), H, zpad).astype(BF16).T)

        wbT[...] = _pk(wqkv_raw[...].T)
        zl = zero_s[0]
        acc = jnp.zeros((DP, A_TQ), F32)
        for t in range(P_NT):
            for ci in A_LAST_SPLIT[t]:
                acc = pv_chunk(sB, sv1, zl, ci, mA_last, acc)
            if t == P_NT - 1:
                finish_A(A_NIT - 1, acc)
            store_x(t, out_proj(woAT, t))
        for t in range(P_NT):
            xnB[t] = layernorm_T(load_x(t))
        proj_B(0)

        def proj_B_body(t, c):
            proj_B(t)
            return c

        lax.fori_loop(1, P_NT, proj_B_body, 0)

        m_last = attn_B_main()

        @pl.when(r_idx == 1)
        def _():
            for i in range(len(OUT_CHUNKS)):
                out_copy(i).wait()

        woBT[...] = _pk(_repitch(woB_raw[...].astype(F32), H, zpad).astype(BF16).T)
        zl = zero_s[0]
        for i, (b0, nb) in enumerate(OUT_CHUNKS):
            for h in B_LAST_SPLIT[i]:
                pv_B(NB - 1, zl, sD, h, m_last[h])
            o = _up(jnp.concatenate([oT[b0 + j] for j in range(nb)], axis=1))
            xs = jnp.concatenate([xT[b0 + j] for j in range(nb)], axis=1) + _dot(_up(woBT[...]), o)
            for j in range(nb):
                xT[b0 + j] = xs[:, j * LB:(j + 1) * LB]
            out_stage[:, b0 * LB:(b0 + nb) * LB] = xs.astype(out_stage.dtype)
            out_copy(i).start()
        return carry

    lax.fori_loop(0, 2, rep, 0)
    for i in range(len(OUT_CHUNKS)):
        out_copy(i).wait()


@jax.jit
def pallas_interleave_layers__grouped_kv_mqa__sliding_block__prompt_kernel(
    A_x: jax.Array,
    A_wq: jax.Array,
    A_wk: jax.Array,
    A_wv: jax.Array,
    A_wo: jax.Array,
    B_x: jax.Array,
    B_wqkv: jax.Array,
    B_wo: jax.Array,
):
    del B_x
    any_spec = pl.BlockSpec(memory_space=pl.ANY)
    outT = pl.pallas_call(
        _kernel,
        out_shape=jax.ShapeDtypeStruct((D, S), A_x.dtype),
        in_specs=[any_spec] * 7,
        out_specs=any_spec,
        scratch_shapes=[
            pltpu.VMEM((P_NT, D, P_TB), BF16),
            pltpu.VMEM((D, D), BF16),
            pltpu.VMEM((DH, D), BF16),
            pltpu.VMEM((DH, D), BF16),
            pltpu.VMEM((D, D), BF16),
            pltpu.VMEM((D, 3 * D), BF16),
            pltpu.VMEM((D, D), BF16),
            pltpu.VMEM((D, S), BF16),
            pltpu.VMEM((D // 2 + DP, D), U32),
            pltpu.VMEM((D // 2, HP), U32),
            pltpu.VMEM((3 * D // 2, D), U32),
            pltpu.VMEM((D // 2, HP), U32),
            pltpu.VMEM((NB, D, LB), F32),
            pltpu.VMEM((P_NT, D, P_TB), BF16),
            pltpu.VMEM((NB, HP // 2, LB), U32),
            pltpu.VMEM((S // 2, DP), U32),
            pltpu.VMEM((DQ, S), U32),
            pltpu.VMEM((H, S // 2 + LB, LB), U32),
            pltpu.VMEM((NB + 2, HP // 2, LB), U32),
            pltpu.VMEM((NB, HP // 2, LB), U32),
            pltpu.VMEM((1, S - A_KV, A_TQ), F32),
            pltpu.VMEM((1, S - A_KV, A_TQ), F32),
            pltpu.VMEM((1, A_KV, A_TQ), F32),
            pltpu.VMEM((1, A_KV, A_TQ), F32),
            pltpu.VMEM((A_NIT, DP, A_TQ), F32),
            pltpu.VMEM((DH, A_KV, LB), F32),
            pltpu.VMEM((1, B_R, H * LB), F32),
            pltpu.VMEM((1, B_R, H * LB), F32),
            pltpu.VMEM((B_RB, LB), F32),
            pltpu.VMEM((1, 8, A_TQ), U32),
            pltpu.SMEM((N_ZERO,), jnp.int32),
            pltpu.SemaphoreType.DMA((P_NT + 6,)),
            pltpu.SemaphoreType.DMA((len(OUT_CHUNKS),)),
        ],
        compiler_params=pltpu.CompilerParams(vmem_limit_bytes=100 * 2**20),
    )(A_x[0].T, A_wq, A_wk.T, A_wv.T, A_wo, B_wqkv, B_wo)
    return outT.T[None]
```

```python
import jax
import jax.numpy as jnp
from jax import lax
import jax.experimental.pallas as pl
import jax.experimental.pallas.tpu as pltpu

S = 2048
D = 448
H = 16
DH = 28
DP = 32
HP = H * DP
DQ = DP // 2
W = 256
LB = 128
NB = S // LB
LH = LB // 2
assert W == 2 * LB
EPS = 1e-5
NEG = -1e30
QSCALE = (DH ** -0.5) * 1.4426950408889634

A_TQ = 256
A_NC = S // LB
A_KV = 8 * A_NC
A_QB = [((S - A_KV) * c // A_NC) // 16 * 16 for c in range(A_NC + 1)]
A_LQ = 3
A_DELTA = 5
A_OFF = 6
A_SHIFT = 6
N_ZERO = 64
A_NQ = A_TQ // LB
A_NH = 18
A_NIT = (S // A_TQ) * H
P_TB = 512
P_NB = P_TB // LB
P_NT = S // P_TB
A_PROJ_CHUNKS = ((0, 1), (1, 1), (2, 2), (4, 4), (8, 4), (12, 4))

B_U = 4
B_SB = LB // B_U
B_RB = LB + B_SB
B_R = LB + B_RB
B_LEAD = 3

A_LAST_SPLIT = ((), range(0, 4), range(4, 10), range(10, 16))
OUT_CHUNKS = ((0, 4), (4, 4), (8, 4), (12, 2), (14, 2))
B_LAST_SPLIT = (range(0, 8), range(8, 12), range(12, 16), (), ())

F32 = jnp.float32
U32 = jnp.uint32
BF16 = jnp.bfloat16


def _dot(a, b):
    return jnp.dot(a, b, preferred_element_type=F32)


def _lane(shape):
    return lax.broadcasted_iota(jnp.int32, shape, 1)


def _sel(mask_fn, a, b):
    bu = jnp.zeros_like(a) if b is None else b
    return jnp.where(mask_fn(_lane(a.shape)), a, bu)


def _pk(x):
    return pltpu.bitcast(x, U32)


def _up(u):
    return pltpu.bitcast(u, BF16)


def _repitch(y, n_heads, fill):
    parts = []
    for h in range(n_heads):
        parts += [y[h * DH:(h + 1) * DH], fill]
    return jnp.concatenate(parts, axis=0)


def _kernel(xT_hbm, wq_hbm, wkT_hbm, wvT_hbm, woA_hbm, wqkv_hbm, woB_hbm, out_hbm,
            x_raw, wq_raw, wkT_raw, wvT_raw, woA_raw, wqkv_raw, woB_raw, out_stage,
            waT, woAT, wbT, woBT,
            xT, xnB, qT, kA, vTA, kB, vTB, oT, sA, sB, sv0, sv1, q32, kb, sC, sD, bias,
            zero_v, zero_s, sems, osems):
    def x_copy(t):
        return pltpu.make_async_copy(xT_hbm.at[:, pl.ds(t * P_TB, P_TB)], x_raw.at[t], sems.at[t])

    w_copies = [
        pltpu.make_async_copy(src, dst, sems.at[P_NT + i])
        for i, (src, dst) in enumerate([
            (wq_hbm, wq_raw), (wkT_hbm, wkT_raw), (wvT_hbm, wvT_raw),
            (woA_hbm, woA_raw), (wqkv_hbm, wqkv_raw), (woB_hbm, woB_raw)])
    ]
    for cp in w_copies[:3]:
        cp.start()
    for t in range(P_NT):
        x_copy(t).start()

    for i in range(N_ZERO):
        zero_s[i] = 0
    zero_v[...] = jnp.zeros(zero_v.shape, U32)

    r = lax.broadcasted_iota(jnp.int32, (B_RB, LB), 0)
    c = lax.broadcasted_iota(jnp.int32, (B_RB, LB), 1)
    use_new = (c // B_SB) >= (r // B_SB)
    ok = jnp.logical_or(jnp.logical_and(use_new, r <= c),
                        jnp.logical_and(jnp.logical_not(use_new), r - B_SB > c))
    bias[...] = jnp.where(ok, 0.0, NEG).astype(F32)
    null_k = jnp.where(_lane((2 * LB, LB)) % DP == DH, NEG, 0.0).astype(BF16)
    for h in range(H):
        kB[h, 0:LB, :] = _pk(null_k)
    vTB[0:2] = jnp.zeros((2, HP // 2, LB), U32)

    def fills(n):
        return (jnp.zeros((DP - DH, n), F32),
                (lax.broadcasted_iota(jnp.int32, (DP - DH, n), 0) == 0).astype(F32))

    zero_fill, one_fill = fills(P_TB)

    def load_x(t):
        return jnp.concatenate([xT[t * P_NB + i] for i in range(P_NB)], axis=1)

    def store_x(t, xs):
        for i in range(P_NB):
            xT[t * P_NB + i] = xs[:, i * LB:(i + 1) * LB]

    def colsum(a):
        if a.shape[1] > LB:
            return jnp.sum(a, axis=0, keepdims=True)
        parts = [a[i * 8:(i + 1) * 8] for i in range(a.shape[0] // 8)]
        while len(parts) > 1:
            parts = ([parts[i] + parts[i + 1] for i in range(0, len(parts) - 1, 2)]
                     + ([parts[-1]] if len(parts) % 2 else []))
        return jnp.sum(parts[0], axis=0, keepdims=True)

    def layernorm_T(xs):
        m = colsum(xs) * (1.0 / D)
        xc = xs - m
        v = colsum(xc * xc) * (1.0 / D)
        return (xc * lax.rsqrt(v + EPS)).astype(BF16)

    def out_proj(wo_ref, t):
        o = _up(jnp.concatenate([oT[t * P_NB + i] for i in range(P_NB)], axis=1))
        return load_x(t) + _dot(_up(wo_ref[...]), o)

    def proj_A(b0, nb):
        n = nb * LB
        zf, of = fills(n)
        xn = layernorm_T(jnp.concatenate([xT[b0 + i] for i in range(nb)], axis=1))
        y = _dot(_up(waT[...]), xn)
        qf = _repitch(y[:D] * QSCALE, H, zf)
        q = _pk(qf.astype(BF16))
        for i in range(nb):
            qT[b0 + i] = q[:, i * LB:(i + 1) * LB]
            bb = b0 + i
            q32[(bb // A_NQ) * H:(bb // A_NQ + 1) * H, :, (bb % A_NQ) * LB:(bb % A_NQ + 1) * LB] = (
                qf[:, i * LB:(i + 1) * LB].reshape(H, DP, LB))
        kA[b0 * LB // 2:(b0 * LB + n) // 2, :] = _pk(y[D:D + DP].T.astype(BF16))
        if b0 == 0:
            for d in range(DH):
                kb[d] = jnp.broadcast_to(y[D + d:D + d + 1, 0:A_KV], (LB, A_KV)).T
        v = _repitch(y[D + DP:D + DP + DH], 1, of)
        vTA[:, b0 * LB:b0 * LB + n] = _pk(v.astype(BF16))

    neg_A = jnp.full((8, A_TQ), -jnp.inf, F32)
    svs = (sv0, sv1)

    def zero_of(x, z):
        return lax.bitcast_convert_type(x, U32) & zero_v[z]

    def qk_chunk(qu, s_ref, ci, m):
        lo, hi = A_QB[ci], A_QB[ci + 1]
        s = _dot(_up(kA[(A_KV + lo) // 2:(A_KV + hi) // 2, :]), _up(qu))
        s_ref[0, lo:hi, :] = s
        mm = jnp.max(s.reshape((hi - lo) // 8, 8, A_TQ), axis=0)
        return jnp.maximum(m, mm), mm

    def qk_head_mxu(it):
        s = _dot(_up(kA[0:A_KV // 2, :]), _up(q_blk(it)))
        svs[it % 2][0] = s
        return jnp.max(s.reshape(A_KV // 8, 8, A_TQ), axis=0)

    def qk_piece(it, zi, sv_ref, p, rel, z):
        qi = it + zero_s[zi]
        accs = [None] * A_NQ
        if rel is not None:
            zz = lax.bitcast_convert_type(zero_of(rel, z), F32)
            accs = [zz[:, l * LB:(l + 1) * LB] for l in range(A_NQ)]
        for d in range(DH):
            kd = kb[d, p * 8:(p + 1) * 8, :]
            for l in range(A_NQ):
                t = kd * q32[qi, d:d + 1, l * LB:(l + 1) * LB]
                accs[l] = t if accs[l] is None else accs[l] + t
        s = jnp.concatenate(accs, axis=1)
        sv_ref[0, p * 8:(p + 1) * 8, :] = s
        return s

    def pv_chunk(s_ref, sv_ref, z, ci, mrow, acc):
        s = sv_ref[z] if ci == 0 else s_ref[z, (ci - 1) * LB:ci * LB, :]
        p = jnp.exp2(s - mrow).astype(BF16)
        return acc + _dot(_up(vTA[:, ci * LB:(ci + 1) * LB]), p)

    def a_index(it):
        if isinstance(it, int):
            return (it // H) * A_NQ, it % H
        return lax.shift_right_logical(it, 4) * A_NQ, it & (H - 1)

    def a_rows(h):
        return pl.ds(h * DQ if isinstance(h, int) else pl.multiple_of(h * DQ, DQ), DQ)

    def q_blk(it):
        qb, h = a_index(it)
        return jnp.concatenate([qT[qb + i, a_rows(h), :] for i in range(A_NQ)], axis=1)

    def finish_A(it, acc):
        qb, h = a_index(it)
        o = _pk((acc * (1.0 / acc[DH:DH + 1, :])).astype(BF16))
        for i in range(A_NQ):
            oT[qb + i, a_rows(h), :] = o[:, i * LB:(i + 1) * LB]

    def steps_A(it0, par, n_steps, m8, mv_acc, first_piece):
        z = zero_s[0]
        gates = {}

        def run_piece(r, rel):
            if not (first_piece <= r < n_steps * A_NC - A_SHIFT):
                return
            n = r + 2 * A_NC - A_OFF
            blk, p = n // A_NC, n % A_NC
            it = it0 + blk
            it = min(it, A_NIT - 1) if isinstance(it, int) else jnp.minimum(it, A_NIT - 1)
            x = qk_piece(it, 1 + n % (N_ZERO - 1), svs[(par + blk) % 2], p, rel, z)
            mv_acc[blk] = x if blk not in mv_acc else jnp.maximum(mv_acc[blk], x)
            gates[r] = x

        for r in range(-A_SHIFT, 0):
            run_piece(r, None)
        for u in range(n_steps):
            it = it0 + u
            s_cur, s_nxt = (sA, sB) if (par + u) % 2 == 0 else (sB, sA)
            sv_cur = svs[(par + u) % 2]
            mrow = jnp.max(m8, axis=0, keepdims=True)
            qn = q_blk(it + 1)
            m = neg_A
            acc = jnp.zeros((DP, A_TQ), F32)
            for c in range(A_NC + A_LQ):
                if c < A_NC:
                    g = u * A_NC + c
                    qu = qn
                    if (g - A_DELTA) in gates:
                        qu = jnp.concatenate(
                            [qn[0:8] | zero_of(gates[g - A_DELTA], z), qn[8:DQ]], axis=0)
                    m, mm = qk_chunk(qu, s_nxt, c, m)
                    run_piece(g, mm)
                if c >= A_LQ:
                    acc = pv_chunk(s_cur, sv_cur, z, c - A_LQ, mrow, acc)
            finish_A(it, acc)
            m8 = jnp.maximum(m, mv_acc[u + 1])
        return m8, mv_acc[n_steps + 1]

    def attn_A_main():
        q0 = q_blk(0)
        m = qk_head_mxu(0)
        for ci in range(A_NC):
            m, _ = qk_chunk(q0, sA, ci, m)
        carry = steps_A(0, 0, 1, m, {1: qk_head_mxu(1)}, A_OFF)

        def body(j, carry):
            return steps_A(A_NH * j + 1, 1, A_NH, carry[0], {1: carry[1]}, -A_SHIFT)

        m_last, _ = lax.fori_loop(0, (A_NIT - 2) // A_NH, body, carry)
        return jnp.max(m_last, axis=0, keepdims=True)

    def proj_B(t):
        xn = xnB[t]
        yq = _dot(_up(wbT[0:D // 2, :]), xn)
        q = _pk(_repitch(yq * QSCALE, H, one_fill).astype(BF16))
        for i in range(P_NB):
            qT[t * P_NB + i] = q[:, i * LB:(i + 1) * LB]
        yk = _dot(_up(wbT[D // 2:D, :]), xn)
        if isinstance(t, int):
            krows = pl.ds(LB + t * (P_TB // 2), P_TB // 2)
        else:
            krows = pl.ds(pl.multiple_of(LB + t * (P_TB // 2), LB), P_TB // 2)
        for h in range(H):
            kh = jnp.concatenate([yk[h * DH:(h + 1) * DH], zero_fill] * B_U, axis=0)
            kB[h, krows, :] = _pk(kh.T.astype(BF16))
        v = _pk(_repitch(_dot(_up(wbT[D:3 * D // 2, :]), xn), H, one_fill).astype(BF16))
        for i in range(P_NB):
            vTB[2 + t * P_NB + i] = v[:, i * LB:(i + 1) * LB]

    lane_p = _lane((B_SB, LB)) // B_SB

    def qk_B(b, s_ref, h, first=0):
        q = qT[b, h * DQ:(h + 1) * DQ, :]
        wq = _up(jnp.concatenate(
            [_sel(lambda ln, u=u: ln // B_SB == u, q, None) for u in range(B_U)], axis=0))
        cols = slice(h * LB, (h + 1) * LB)

        def k_blk(i):
            if first:
                return kB[h, (b + i) * LH:(b + i + 1) * LH, :]
            return kB[h, pl.ds(pl.multiple_of((b + i) * LH, LH), LH), :]

        k_old, k_new = k_blk(0), k_blk(2)
        sh = B_SB // 2
        rows = [k_new[0:sh]]
        for rr in range(B_U - 1):
            rows.append(_sel(lambda ln, rr=rr: ln // DP <= rr,
                             k_old[rr * sh:(rr + 1) * sh], k_new[(rr + 1) * sh:(rr + 2) * sh]))
        if not first:
            rows.append(k_old[(B_U - 1) * sh:])
        nr = len(rows) * B_SB
        s2 = _dot(_up(jnp.concatenate(rows, axis=0)), wq) + bias[0:nr, :]
        s_ref[0, LB:LB + nr, cols] = s2
        mm = jnp.max(s2.reshape(nr // 8, 8, LB), axis=0)
        if first != 1:
            s1 = _dot(_up(k_blk(1)), wq)
            s_ref[0, 0:LB, cols] = s1
            mm = jnp.maximum(mm, jnp.max(s1.reshape(LB // 8, 8, LB), axis=0))
        if first == 2:
            s_ref[0, 2 * LB:B_R, cols] = jnp.full((B_SB, LB), NEG, F32)
        return jnp.max(mm, axis=0, keepdims=True)

    def pv_B(b, z, s_ref, h, mrow, first=False):
        def ex(lo, hi):
            return jnp.exp2(s_ref[z, lo:hi, h * LB:(h + 1) * LB] - mrow)

        rows = slice(h * DQ, (h + 1) * DQ)
        news = [ex(LB, LB + B_SB)]
        olds = []
        for rr in range(B_U - 1):
            px = ex(LB + (rr + 1) * B_SB, LB + (rr + 2) * B_SB)
            olds.append(jnp.where(lane_p <= rr, px, 0.0))
            news.append(jnp.where(lane_p > rr, px, 0.0))
        acc = _dot(_up(vTB[b + 2, rows, :]), jnp.concatenate(news, axis=0).astype(BF16))
        if not first:
            olds.append(ex(2 * LB, B_R))
            acc = (acc + _dot(_up(vTB[b + 1, rows, :]), ex(0, LB).astype(BF16))
                   + _dot(_up(vTB[b, rows, :]), jnp.concatenate(olds, axis=0).astype(BF16)))
        oT[b, rows, :] = _pk((acc * (1.0 / acc[DH:DH + 1, :])).astype(BF16))

    def step_B(b, z, mrows, s_cur, s_nxt, first=False):
        m = []
        for h in range(H + B_LEAD):
            if h < H:
                m.append(qk_B(b + 1, s_nxt, h, first=2 if first else 0))
            if h >= B_LEAD:
                pv_B(b, z, s_cur, h - B_LEAD, mrows[h - B_LEAD], first=first)
        return tuple(m)

    def attn_B_main():
        m0 = tuple(qk_B(0, sC, h, first=1) for h in range(H))
        m1 = step_B(0, zero_s[0], m0, sC, sD, first=True)

        def body(jj, mrows):
            z = zero_s[0]
            mrows = step_B(2 * jj + 1, z, mrows, sD, sC)
            return step_B(2 * jj + 2, z, mrows, sC, sD)

        return lax.fori_loop(0, (NB - 2) // 2, body, m1)

    zpad = jnp.zeros((DP - DH, D), F32)
    for cp in w_copies[:3]:
        cp.wait()
    waT[0:D // 2, :] = _pk(wq_raw[...].T)
    waT[D // 2:D // 2 + DP, :] = _pk(jnp.concatenate(
        [wkT_raw[...].astype(F32), zpad, wvT_raw[...].astype(F32), zpad], axis=0).astype(BF16))
    for t in range(P_NT):
        x_copy(t).wait()
        store_x(t, x_raw[t].astype(F32))
    for cp in w_copies[3:]:
        cp.start()

    def out_copy(i):
        cols = pl.ds(OUT_CHUNKS[i][0] * LB, OUT_CHUNKS[i][1] * LB)
        return pltpu.make_async_copy(out_stage.at[:, cols], out_hbm.at[:, cols], osems.at[i])

    def rep(r_idx, carry):
        for b0, nb in A_PROJ_CHUNKS:
            proj_A(b0, nb)

        mA_last = attn_A_main()

        @pl.when(r_idx == 0)
        def _():
            for cp in w_copies[3:]:
                cp.wait()
            woAT[...] = _pk(_repitch(woA_raw[...].astype(F32), H, zpad).astype(BF16).T)

        wbT[...] = _pk(wqkv_raw[...].T)
        zl = zero_s[0]
        acc = jnp.zeros((DP, A_TQ), F32)
        for t in range(P_NT):
            for ci in A_LAST_SPLIT[t]:
                acc = pv_chunk(sB, sv1, zl, ci, mA_last, acc)
            if t == P_NT - 1:
                finish_A(A_NIT - 1, acc)
            store_x(t, out_proj(woAT, t))
        for t in range(P_NT):
            xnB[t] = layernorm_T(load_x(t))
        proj_B(0)

        def proj_B_body(t, c):
            proj_B(t)
            return c

        lax.fori_loop(1, P_NT, proj_B_body, 0)

        m_last = attn_B_main()

        @pl.when(r_idx == 1)
        def _():
            for i in range(len(OUT_CHUNKS)):
                out_copy(i).wait()

        woBT[...] = _pk(_repitch(woB_raw[...].astype(F32), H, zpad).astype(BF16).T)
        zl = zero_s[0]
        for i, (b0, nb) in enumerate(OUT_CHUNKS):
            for h in B_LAST_SPLIT[i]:
                pv_B(NB - 1, zl, sD, h, m_last[h])
            o = _up(jnp.concatenate([oT[b0 + j] for j in range(nb)], axis=1))
            xs = jnp.concatenate([xT[b0 + j] for j in range(nb)], axis=1) + _dot(_up(woBT[...]), o)
            for j in range(nb):
                xT[b0 + j] = xs[:, j * LB:(j + 1) * LB]
            out_stage[:, b0 * LB:(b0 + nb) * LB] = xs.astype(out_stage.dtype)
            out_copy(i).start()
        return carry

    lax.fori_loop(0, 2, rep, 0)
    for i in range(len(OUT_CHUNKS)):
        out_copy(i).wait()


@jax.jit
def pallas_interleave_layers__grouped_kv_mqa__sliding_block__prompt_kernel(
    A_x: jax.Array,
    A_wq: jax.Array,
    A_wk: jax.Array,
    A_wv: jax.Array,
    A_wo: jax.Array,
    B_x: jax.Array,
    B_wqkv: jax.Array,
    B_wo: jax.Array,
):
    del B_x
    any_spec = pl.BlockSpec(memory_space=pl.ANY)
    outT = pl.pallas_call(
        _kernel,
        out_shape=jax.ShapeDtypeStruct((D, S), A_x.dtype),
        in_specs=[any_spec] * 7,
        out_specs=any_spec,
        scratch_shapes=[
            pltpu.VMEM((P_NT, D, P_TB), BF16),
            pltpu.VMEM((D, D), BF16),
            pltpu.VMEM((DH, D), BF16),
            pltpu.VMEM((DH, D), BF16),
            pltpu.VMEM((D, D), BF16),
            pltpu.VMEM((D, 3 * D), BF16),
            pltpu.VMEM((D, D), BF16),
            pltpu.VMEM((D, S), BF16),
            pltpu.VMEM((D // 2 + DP, D), U32),
            pltpu.VMEM((D // 2, HP), U32),
            pltpu.VMEM((3 * D // 2, D), U32),
            pltpu.VMEM((D // 2, HP), U32),
            pltpu.VMEM((NB, D, LB), F32),
            pltpu.VMEM((P_NT, D, P_TB), BF16),
            pltpu.VMEM((NB, HP // 2, LB), U32),
            pltpu.VMEM((S // 2, DP), U32),
            pltpu.VMEM((DQ, S), U32),
            pltpu.VMEM((H, S // 2 + LB, LB), U32),
            pltpu.VMEM((NB + 2, HP // 2, LB), U32),
            pltpu.VMEM((NB, HP // 2, LB), U32),
            pltpu.VMEM((1, S - A_KV, A_TQ), F32),
            pltpu.VMEM((1, S - A_KV, A_TQ), F32),
            pltpu.VMEM((1, A_KV, A_TQ), F32),
            pltpu.VMEM((1, A_KV, A_TQ), F32),
            pltpu.VMEM((A_NIT, DP, A_TQ), F32),
            pltpu.VMEM((DH, A_KV, LB), F32),
            pltpu.VMEM((1, B_R, H * LB), F32),
            pltpu.VMEM((1, B_R, H * LB), F32),
            pltpu.VMEM((B_RB, LB), F32),
            pltpu.VMEM((1, 8, A_TQ), U32),
            pltpu.SMEM((N_ZERO,), jnp.int32),
            pltpu.SemaphoreType.DMA((P_NT + 6,)),
            pltpu.SemaphoreType.DMA((len(OUT_CHUNKS),)),
        ],
        compiler_params=pltpu.CompilerParams(vmem_limit_bytes=100 * 2**20),
    )(A_x[0].T, A_wq, A_wk.T, A_wv.T, A_wo, B_wqkv, B_wo)
    return outT.T[None]
```
